```python
import jax
import jax.numpy as jnp

def _softmax(x, axis=-1):
    return jax.nn.softmax(x, axis=axis)

def _gelu(x):
    return jax.nn.gelu(x, approximate=True)

def _silu(x):
    return jax.nn.silu(x)

def _sigmoid(x):
    return jax.nn.sigmoid(x)

def _layernorm(x, axis=-1, eps=1e-05):
    m = jnp.mean(x, axis=axis, keepdims=True)
    v = jnp.var(x, axis=axis, keepdims=True)
    return (x - m) / jnp.sqrt(v + eps)

def _scatter_add(tgt, idx, src, axis=0):
    return tgt.at[idx].add(src)

def _segment_sum(src, seg, n):
    return jax.ops.segment_sum(src, seg, n)

class _Rng:

    def __init__(self, key):
        self._k = key

    def _next(self):
        self._k, sub = jax.random.split(self._k)
        return sub

    def normal(self, shape):
        return jax.random.normal(self._next(), shape, dtype=jnp.bfloat16)

    def randint(self, lo, hi, shape):
        return jax.random.randint(self._next(), shape, lo, hi, dtype=jnp.int32)

    def uniform(self, shape, lo=0.0, hi=1.0):
        return jax.random.uniform(self._next(), shape, jnp.bfloat16, lo, hi)

    def permutation(self, n):
        return jax.random.permutation(self._next(), n)
kernel_name = 'gated_mix__memory_aug_recurrent_mem_tr__mixer_s_mlp__prompt'

def setup_inputs():
    _rng = _Rng(jax.random.key(int.from_bytes(__import__("os").urandom(4), "little")))
    _w = lambda a: (lambda t: t.astype(jnp.bfloat16) if jnp.issubdtype(t.dtype, jnp.floating) else t)(jnp.asarray(a))

    def _A_setup():
        B, S, Dm = (1, 2048, 1024)
        H, Dh = (32, 128)
        M, seg = (8, 32)
        seg = min(seg, S)
        S = S // seg * seg
        return {'x': _w((lambda *s: _rng.normal(s) * 0.05)(B, S, Dm)), 'mem0': _w((lambda *s: _rng.normal(s) * 0.05)(B, M, Dm)), 'Wq': _w((lambda *s: _rng.normal(s) * 0.05)(Dm, H, Dh) * Dm ** (-0.5)), 'Wk': _w((lambda *s: _rng.normal(s) * 0.05)(Dm, H, Dh) * Dm ** (-0.5)), 'Wv': _w((lambda *s: _rng.normal(s) * 0.05)(Dm, H, Dh) * Dm ** (-0.5)), 'Wo': _w((lambda *s: _rng.normal(s) * 0.05)(H, Dh, Dm) * (H * Dh) ** (-0.5)), 'seg_len': seg}
    _A_in = _A_setup()

    def _B_setup():
        B, S, D, F = (1, 2048, 1024, 3584)
        return {'x': _w((lambda *s: _rng.normal(s) * 0.05)(B, S, D)), 'w1': _w((lambda *s: _rng.normal(s) * 0.05)(D, D) * D ** (-0.5)), 'w2': _w((lambda *s: _rng.normal(s) * 0.05)(D, D) * D ** (-0.5)), 'w3': _w((lambda *s: _rng.normal(s) * 0.05)(D, F) * D ** (-0.5)), 'w4': _w((lambda *s: _rng.normal(s) * 0.05)(F, D) * F ** (-0.5))}
    _B_in = _B_setup()
    return {'A_x': _A_in['x'], 'A_mem0': _A_in['mem0'], 'A_Wq': _A_in['Wq'], 'A_Wk': _A_in['Wk'], 'A_Wv': _A_in['Wv'], 'A_Wo': _A_in['Wo'], 'A_seg_len': _A_in['seg_len'], 'B_x': _B_in['x'], 'B_w1': _B_in['w1'], 'B_w2': _B_in['w2'], 'B_w3': _B_in['w3'], 'B_w4': _B_in['w4'], 'gate_w': _w((lambda *s: _rng.normal(s) * 0.05)(1024))}

def reference(A_x, A_mem0, A_Wq, A_Wk, A_Wv, A_Wo, A_seg_len, B_x, B_w1, B_w2, B_w3, B_w4, gate_w):

    def _A_ref(x, mem0, Wq, Wk, Wv, Wo, seg_len):
        B, S, Dm = x.shape
        H, Dh = (Wq.shape[1], Wq.shape[2])
        M = mem0.shape[1]
        scale = Dh ** (-0.5)
        n_seg = S // seg_len
        L = M + seg_len
        idx = jnp.arange(L)
        mask = (idx[:, None] < M) | (idx[:, None] >= idx[None, :])
        mem = mem0
        outs = []
        for s in range(n_seg):
            xs = x[:, s * seg_len:(s + 1) * seg_len, :].copy()
            h = jnp.concatenate([mem, xs], axis=1)
            q = jnp.einsum('btd,dhe->bhte', h, Wq)
            k = jnp.einsum('btd,dhe->bhte', h, Wk)
            v = jnp.einsum('btd,dhe->bhte', h, Wv)
            scores = jnp.einsum('bhqe,bhke->bhqk', q, k) * scale
            scores = jnp.where(mask[None, None], scores, -1000000000.0)
            p = _softmax(scores, axis=-1)
            o = jnp.einsum('bhqk,bhke->bhqe', p, v)
            o = jnp.einsum('bhte,hed->btd', o, Wo)
            mem = o[:, :M, :].copy()
            outs.append(o[:, M:, :])
        return jnp.concatenate(outs, axis=1)

    def _B_ref(x, w1, w2, w3, w4):
        B, S, D = x.shape
        h = _gelu(_layernorm(x, axis=-1) @ w1)
        c = D // 4
        g0 = jnp.pad(h[:, :, 0 * c:1 * c], ((0, 0), (1, 0), (0, 0)))[:, :S, :]
        g1 = jnp.pad(h[:, :, 1 * c:2 * c], ((0, 0), (0, 1), (0, 0)))[:, 1:, :]
        g2 = jnp.pad(h[:, :, 2 * c:3 * c], ((0, 0), (2, 0), (0, 0)))[:, :S, :]
        g3 = jnp.pad(h[:, :, 3 * c:], ((0, 0), (0, 2), (0, 0)))[:, 2:, :]
        hs = jnp.concatenate([g0, g1, g2, g3], axis=-1) @ w2
        x1 = x + hs
        h2 = _gelu(_layernorm(x1, axis=-1) @ w3) @ w4
        return x1 + h2
    x = A_x
    g = _sigmoid((x * gate_w).sum(-1, keepdims=True))
    a = _A_ref(x, A_mem0, A_Wq, A_Wk, A_Wv, A_Wo, A_seg_len)
    b = _B_ref(x, B_w1, B_w2, B_w3, B_w4)
    return g * a + (1 - g) * b
```

```python
import functools
import math

import jax
import jax.numpy as jnp
from jax import lax
import jax.experimental.pallas as pl
import jax.experimental.pallas.tpu as pltpu

F32 = jnp.float32
BF16 = jnp.bfloat16
LANES = 128
LOG2E = 1.4426950408889634


def _dot(a, b):
    return lax.dot_general(a, b, (((1,), (0,)), ((), ())), preferred_element_type=F32)


def _dot_nt(a, b):
    return lax.dot_general(a, b, (((1,), (1,)), ((), ())), preferred_element_type=F32)


def _layernorm(x, eps=1e-5):
    m = jnp.mean(x, axis=-1, keepdims=True)
    xc = x - m
    v = jnp.mean(xc * xc, axis=-1, keepdims=True)
    return xc * lax.rsqrt(v + eps)


def _gelu(x):
    c = math.sqrt(2.0 / math.pi)
    return 0.5 * x * (1.0 + jnp.tanh(c * (x + 0.044715 * (x * x * x))))


def _kernel(x_hbm, mem0_ref, wq_hbm, wk_hbm, wv_hbm, wo_hbm, w1_hbm, w2_hbm, w3_hbm, w4_hbm, gw_ref,
            out_hbm,
            x_v, wqkv_v, wo_v, w1_v, w2_v, w3_v, w4_v, stage_v, h_v, bb_v, g_v, out_v, sems, osems,
            *, S, D, H, Dh, M, SEG, TB):
    NSEG = S // SEG
    NT = S // TB
    DC = D // NT
    C = D // 4
    HALO = 8

    cp_x = pltpu.make_async_copy(x_hbm, x_v, sems.at[0])
    cp_w1 = pltpu.make_async_copy(w1_hbm, w1_v, sems.at[1])
    cp_w2 = pltpu.make_async_copy(w2_hbm, w2_v, sems.at[2])
    cp_w3 = pltpu.make_async_copy(w3_hbm, w3_v, sems.at[3])
    cp_w4 = pltpu.make_async_copy(w4_hbm, w4_v, sems.at[4])
    cp_qkv = [pltpu.make_async_copy(w, stage_v.at[i], sems.at[5 + i])
              for i, w in enumerate((wq_hbm, wk_hbm, wv_hbm))]
    cp_wo = [pltpu.make_async_copy(wo_hbm.at[:, pl.ds(j * LANES, LANES)], wo_v.at[j], sems.at[8 + j])
             for j in range(D // LANES)]
    cp_x.start()
    cp_w1.start()
    cp_w2.start()
    cp_w3.start()
    cp_w4.start()
    for c in cp_qkv:
        c.start()
    for c in cp_wo:
        c.start()

    h_v[0:HALO, :] = jnp.zeros((HALO, D), F32)
    h_v[HALO + S:HALO + S + HALO, :] = jnp.zeros((HALO, D), F32)
    cp_x.wait()
    cp_w1.wait()

    def b_pass1(i, _):
        r0 = pl.multiple_of(i * TB, TB)
        xt = x_v[pl.ds(r0, TB), :].astype(F32)
        g = jax.nn.sigmoid(jnp.sum(xt * gw_ref[...].astype(F32), axis=-1, keepdims=True))
        g_v[pl.ds(r0, TB), :] = jnp.broadcast_to(g, (TB, LANES))
        hh = _gelu(_dot(_layernorm(xt).astype(BF16), w1_v[...]))
        h_v[pl.ds(r0 + HALO, TB), :] = hh
        return 0

    lax.fori_loop(0, NT, b_pass1, 0)

    cp_w2.wait()
    cp_w3.wait()
    cp_w4.wait()
    for c in cp_qkv:
        c.wait()

    stage_u = stage_v.bitcast(jnp.uint32)

    def b_pass2(i, _):
        r0 = pl.multiple_of(i * TB, TB)
        win = h_v[pl.ds(r0, TB + 2 * HALO), :]
        hs_in = jnp.concatenate([
            win[HALO - 1:HALO - 1 + TB, 0 * C:1 * C],
            win[HALO + 1:HALO + 1 + TB, 1 * C:2 * C],
            win[HALO - 2:HALO - 2 + TB, 2 * C:3 * C],
            win[HALO + 2:HALO + 2 + TB, 3 * C:4 * C]], axis=1).astype(BF16)
        x1 = x_v[pl.ds(r0, TB), :].astype(F32) + _dot(hs_in, w2_v[...])
        u = _gelu(_dot(_layernorm(x1).astype(BF16), w3_v[...])).astype(BF16)
        b = x1 + _dot(u, w4_v[...])
        g = g_v[pl.ds(r0, TB), :]
        bb_v[pl.ds(r0, TB), :] = (1.0 - g[:, 0:1]) * b

        d0 = pl.multiple_of(i * DC, DC)
        u0 = pl.multiple_of(i * (DC * H // 2), DC * H // 2)
        for m in range(3):
            chunk = stage_u.at[m, pl.ds(u0, DC * H // 2), :]
            for p in range(H // 2):
                w = chunk[pl.ds(p, DC, stride=H // 2), :]
                lo = pltpu.bitcast(w << 16, F32).astype(BF16)
                hi = pltpu.bitcast(w & jnp.uint32(0xFFFF0000), F32).astype(BF16)
                wqkv_v[m * H + 2 * p, pl.ds(d0, DC), :] = lo
                wqkv_v[m * H + 2 * p + 1, pl.ds(d0, DC), :] = hi
        return 0

    lax.fori_loop(0, NT, b_pass2, 0)

    for c in cp_wo:
        c.wait()

    L = M + SEG
    LP = (L + 15) // 16 * 16
    row = lax.broadcasted_iota(jnp.int32, (L, LP), 0)
    col = lax.broadcasted_iota(jnp.int32, (L, LP), 1)
    mask = jnp.logical_and(jnp.logical_or(row < M, row >= col), col < L)
    fill = jnp.where(col < L, -1e9 * LOG2E, -jnp.inf).astype(F32)
    qk_scale = (Dh ** -0.5) * LOG2E
    zpad = jnp.zeros((LP - L, Dh), F32)

    def out_copy(s):
        r0 = pl.multiple_of(s * SEG, SEG)
        return pltpu.make_async_copy(out_v.at[pl.ds(r0, SEG), :], out_hbm.at[pl.ds(r0, SEG), :], osems.at[0])

    def seg_step(s, mem):
        r0 = pl.multiple_of(s * SEG, SEG)
        hcat = jnp.concatenate([mem, x_v[pl.ds(r0, SEG), :].astype(F32)], axis=0)

        def project(h):
            return (_dot(hcat, wqkv_v[h]), _dot(hcat, wqkv_v[H + h]), _dot(hcat, wqkv_v[2 * H + h]))

        def attend(q, k, v):
            kp = jnp.concatenate([k, zpad], axis=0).astype(BF16)
            vp = jnp.concatenate([v, zpad], axis=0).astype(BF16)
            t = jnp.where(mask, _dot_nt(q, kp) * qk_scale, fill)
            p = jnp.exp2(t - jnp.max(t, axis=-1, keepdims=True))
            l = jnp.sum(p, axis=-1, keepdims=True)
            r = pl.reciprocal(l, approx=True)
            r = r * (2.0 - l * r)
            return _dot(p * r, vp)

        outs = []
        nxt = project(0)
        for h in range(H):
            cur = nxt
            if h + 1 < H:
                nxt = project(h + 1)
            outs.append(attend(*cur))
        o = jnp.concatenate(outs, axis=1)
        res = jnp.concatenate([_dot(o, wo_v[j]) for j in range(D // LANES)], axis=1)
        g = g_v[pl.ds(r0, SEG), :]
        out_v[pl.ds(r0, SEG), :] = (g[:, 0:1] * res[M:] + bb_v[pl.ds(r0, SEG), :]).astype(BF16)
        return res[:M]

    lax.fori_loop(0, NSEG, seg_step, mem0_ref[...].astype(F32))

    cp_out = pltpu.make_async_copy(out_v, out_hbm, osems.at[0])
    cp_out.start()
    cp_out.wait()


@functools.partial(jax.jit, static_argnames=("A_seg_len",))
def pallas_gated_mix__memory_aug_recurrent_mem_tr__mixer_s_mlp__prompt_kernel(
    A_x: jax.Array,
    A_mem0: jax.Array,
    A_Wq: jax.Array,
    A_Wk: jax.Array,
    A_Wv: jax.Array,
    A_Wo: jax.Array,
    A_seg_len,
    B_x: jax.Array,
    B_w1: jax.Array,
    B_w2: jax.Array,
    B_w3: jax.Array,
    B_w4: jax.Array,
    gate_w: jax.Array,
):
    del B_x
    B, S, D = A_x.shape
    assert B == 1
    _, H, Dh = A_Wq.shape
    M = A_mem0.shape[1]
    SEG = int(A_seg_len)
    Fh = B_w3.shape[1]
    TB = 256

    any_spec = pl.BlockSpec(memory_space=pl.ANY)
    vmem_spec = pl.BlockSpec(memory_space=pltpu.VMEM)
    kernel = functools.partial(_kernel, S=S, D=D, H=H, Dh=Dh, M=M, SEG=SEG, TB=TB)
    out = pl.pallas_call(
        kernel,
        out_shape=jax.ShapeDtypeStruct((S, D), A_x.dtype),
        in_specs=[any_spec, vmem_spec] + [any_spec] * 8 + [vmem_spec],
        out_specs=any_spec,
        scratch_shapes=[
            pltpu.VMEM((S, D), BF16),
            pltpu.VMEM((3 * H, D, Dh), BF16),
            pltpu.VMEM((D // LANES, H * Dh, LANES), BF16),
            pltpu.VMEM((D, D), BF16),
            pltpu.VMEM((D, D), BF16),
            pltpu.VMEM((D, Fh), BF16),
            pltpu.VMEM((Fh, D), BF16),
            pltpu.VMEM((3, D * H, Dh), BF16),
            pltpu.VMEM((S + 16, D), F32),
            pltpu.VMEM((S, D), F32),
            pltpu.VMEM((S, LANES), F32),
            pltpu.VMEM((S, D), BF16),
            pltpu.SemaphoreType.DMA((8 + D // LANES,)),
            pltpu.SemaphoreType.DMA((1,)),
        ],
        compiler_params=pltpu.CompilerParams(vmem_limit_bytes=124 * 1024 * 1024),
    )(
        A_x.reshape(S, D),
        A_mem0.reshape(M, D),
        A_Wq.reshape(D * H, Dh),
        A_Wk.reshape(D * H, Dh),
        A_Wv.reshape(D * H, Dh),
        A_Wo.reshape(H * Dh, D),
        B_w1, B_w2, B_w3, B_w4,
        gate_w.reshape(1, D),
    )
    return out.reshape(B, S, D)
```

```python
import functools
import math

import jax
import jax.numpy as jnp
from jax import lax
import jax.experimental.pallas as pl
import jax.experimental.pallas.tpu as pltpu

F32 = jnp.float32
BF16 = jnp.bfloat16
LANES = 128
LOG2E = 1.4426950408889634


def _dot(a, b):
    return lax.dot_general(a, b, (((1,), (0,)), ((), ())), preferred_element_type=F32)


def _dot_nt(a, b):
    return lax.dot_general(a, b, (((1,), (1,)), ((), ())), preferred_element_type=F32)


def _layernorm(x, eps=1e-5):
    m = jnp.mean(x, axis=-1, keepdims=True)
    xc = x - m
    v = jnp.mean(xc * xc, axis=-1, keepdims=True)
    return xc * lax.rsqrt(v + eps)


def _gelu(x):
    c = math.sqrt(2.0 / math.pi)
    return 0.5 * x * (1.0 + jnp.tanh(c * (x + 0.044715 * (x * x * x))))


def _kernel(x_hbm, mem0_ref, wq_hbm, wk_hbm, wv_hbm, wo_hbm, w1_hbm, w2_hbm, w3_hbm, w4_hbm, gw_ref,
            out_hbm,
            x_v, wqkv_v, wo_v, w1_v, w2_v, w3_v, w4_v, stage_v, h_v, bb_v, g_v, out_v, xsems, qsems, wsems,
            *, S, D, H, Dh, M, SEG, TB):
    NSEG = S // SEG
    NT = S // TB
    DC = D // NT
    C = D // 4
    HALO = 8

    NJ = D // LANES
    UC = DC * H

    def cp_x(i):
        r0 = pl.multiple_of(i * TB, TB)
        return pltpu.make_async_copy(x_hbm.at[pl.ds(r0, TB), :], x_v.at[pl.ds(r0, TB), :], xsems.at[i])

    def cp_qkv(m, i):
        u0 = pl.multiple_of(i * UC, UC)
        w = (wq_hbm, wk_hbm, wv_hbm)[m]
        return pltpu.make_async_copy(w.at[pl.ds(u0, UC), :], stage_v.at[m, pl.ds(u0, UC), :], qsems.at[m * NT + i])

    cp_w1 = pltpu.make_async_copy(w1_hbm, w1_v, wsems.at[0])
    cp_w2 = pltpu.make_async_copy(w2_hbm, w2_v, wsems.at[1])
    cp_w3 = pltpu.make_async_copy(w3_hbm, w3_v, wsems.at[2])
    cp_w4 = pltpu.make_async_copy(w4_hbm, w4_v, wsems.at[3])
    cp_wo = [pltpu.make_async_copy(wo_hbm.at[:, pl.ds(j * LANES, LANES)], wo_v.bitcast(BF16).at[j], wsems.at[4 + j])
             for j in range(NJ)]

    cp_x(0).start()
    cp_w1.start()
    h_v[0:HALO, :] = jnp.zeros((HALO, D), F32)
    h_v[HALO + S:HALO + S + HALO, :] = jnp.zeros((HALO, D), F32)
    cp_w1.wait()
    for i in range(1, NT):
        cp_x(i).start()
    cp_w2.start()
    cp_w3.start()
    cp_w4.start()

    def b_pass1(i, _):
        r0 = pl.multiple_of(i * TB, TB)
        cp_x(i).wait()
        xt = x_v[pl.ds(r0, TB), :].astype(F32)
        g = jax.nn.sigmoid(jnp.sum(xt * gw_ref[...].astype(F32), axis=-1, keepdims=True))
        g_v[pl.ds(r0, TB), :] = jnp.broadcast_to(g, (TB, LANES))
        hh = _gelu(_dot(_layernorm(xt).astype(BF16), w1_v[...]))
        h_v[pl.ds(r0 + HALO, TB), :] = hh
        return 0

    lax.fori_loop(0, NT, b_pass1, 0)

    cp_w2.wait()
    cp_w3.wait()
    cp_w4.wait()
    for i in range(NT):
        for m in range(3):
            cp_qkv(m, i).start()
    for c in cp_wo:
        c.start()

    stage_u = stage_v.bitcast(jnp.uint32)

    def relayout(i):
        d0 = pl.multiple_of(i * (DC // 2), DC // 2)
        u0 = pl.multiple_of(i * (UC // 2), UC // 2)
        for m in range(3):
            chunk = stage_u.at[m, pl.ds(u0, UC // 2), :]
            for p in range(H // 2):
                w = chunk[pl.ds(p, DC, stride=H // 2), :]
                lo = pltpu.bitcast(w << 16, F32).astype(BF16)
                hi = pltpu.bitcast(w & jnp.uint32(0xFFFF0000), F32).astype(BF16)
                wqkv_v[m * H + 2 * p, pl.ds(d0, DC // 2), :] = pltpu.bitcast(lo, jnp.uint32)
                wqkv_v[m * H + 2 * p + 1, pl.ds(d0, DC // 2), :] = pltpu.bitcast(hi, jnp.uint32)

    def b_pass2(i, _):
        r0 = pl.multiple_of(i * TB, TB)
        win = h_v[pl.ds(r0, TB + 2 * HALO), :]
        hs_in = jnp.concatenate([
            win[HALO - 1:HALO - 1 + TB, 0 * C:1 * C],
            win[HALO + 1:HALO + 1 + TB, 1 * C:2 * C],
            win[HALO - 2:HALO - 2 + TB, 2 * C:3 * C],
            win[HALO + 2:HALO + 2 + TB, 3 * C:4 * C]], axis=1).astype(BF16)
        x1 = x_v[pl.ds(r0, TB), :].astype(F32) + _dot(hs_in, w2_v[...])
        u = _gelu(_dot(_layernorm(x1).astype(BF16), w3_v[...])).astype(BF16)
        b = x1 + _dot(u, w4_v[...])
        g = g_v[pl.ds(r0, TB), :]
        bb_v[pl.ds(r0, TB), :] = (1.0 - g[:, 0:1]) * b
        for m in range(3):
            cp_qkv(m, i).wait()
        relayout(i)
        return 0

    lax.fori_loop(0, NT, b_pass2, 0)

    for c in cp_wo:
        c.wait()

    L = M + SEG
    LP = (L + 15) // 16 * 16
    G = 4
    NG = H // G
    row = lax.broadcasted_iota(jnp.int32, (L, LP), 0)
    col = lax.broadcasted_iota(jnp.int32, (L, LP), 1)
    mask = jnp.logical_and(jnp.logical_or(row < M, row >= col), col < L)
    fill = jnp.where(col < L, -1e9 * LOG2E, -jnp.inf).astype(F32)
    qk_scale = (Dh ** -0.5) * LOG2E
    zpad = jnp.zeros((LP - L, Dh), F32)

    def seg_step(s, mem):
        r0 = pl.multiple_of(s * SEG, SEG)
        hcat = jnp.concatenate([mem, x_v[pl.ds(r0, SEG), :].astype(F32)], axis=0)

        def project(m, g):
            return [_dot(hcat, pltpu.bitcast(wqkv_v[m * H + g * G + t], BF16)) for t in range(G)]

        def pad_bf16(ts):
            return [jnp.concatenate([t, zpad], axis=0).astype(BF16) for t in ts]

        def softmax(sc):
            t = jnp.where(mask, sc * qk_scale, fill)
            p = jnp.exp2(t - jnp.max(t, axis=-1, keepdims=True))
            l = jnp.sum(p, axis=-1, keepdims=True)
            r = pl.reciprocal(l, approx=True)
            r = r * (2.0 - l * r)
            return p * r

        def out_proj(g, og):
            ocat = jnp.concatenate(og, axis=1)
            k0 = g * G * Dh // 2
            return [_dot(ocat, pltpu.bitcast(wo_v[j, k0:k0 + G * Dh // 2, :], BF16)) for j in range(NJ)]

        q, k, v, p, o = {}, {}, {}, {}, {}
        acc = None
        WO_LAG = 3
        for g in range(NG + WO_LAG):
            if g < NG:
                q[g] = project(0, g)
            if 0 <= g - 1 < NG:
                p[g - 1] = [softmax(_dot_nt(a, b)) for a, b in zip(q.pop(g - 1), k.pop(g - 1))]
            if g < NG:
                k[g] = pad_bf16(project(1, g))
            if 0 <= g - WO_LAG < NG:
                part = out_proj(g - WO_LAG, o.pop(g - WO_LAG))
                acc = part if acc is None else [a + b for a, b in zip(acc, part)]
            if 0 <= g - 1 < NG:
                o[g - 1] = [_dot(a, b) for a, b in zip(p.pop(g - 1), v.pop(g - 1))]
            if g < NG:
                v[g] = pad_bf16(project(2, g))
        res = jnp.concatenate(acc, axis=1)
        g = g_v[pl.ds(r0, SEG), :]
        out_v[pl.ds(r0, SEG), :] = (g[:, 0:1] * res[M:] + bb_v[pl.ds(r0, SEG), :]).astype(BF16)
        return res[:M]

    lax.fori_loop(0, NSEG, seg_step, mem0_ref[...].astype(F32))

    cp_out = pltpu.make_async_copy(out_v, out_hbm, wsems.at[0])
    cp_out.start()
    cp_out.wait()


@functools.partial(jax.jit, static_argnames=("A_seg_len",))
def pallas_gated_mix__memory_aug_recurrent_mem_tr__mixer_s_mlp__prompt_kernel(
    A_x: jax.Array,
    A_mem0: jax.Array,
    A_Wq: jax.Array,
    A_Wk: jax.Array,
    A_Wv: jax.Array,
    A_Wo: jax.Array,
    A_seg_len,
    B_x: jax.Array,
    B_w1: jax.Array,
    B_w2: jax.Array,
    B_w3: jax.Array,
    B_w4: jax.Array,
    gate_w: jax.Array,
):
    del B_x
    B, S, D = A_x.shape
    assert B == 1
    _, H, Dh = A_Wq.shape
    M = A_mem0.shape[1]
    SEG = int(A_seg_len)
    Fh = B_w3.shape[1]
    TB = 256

    any_spec = pl.BlockSpec(memory_space=pl.ANY)
    vmem_spec = pl.BlockSpec(memory_space=pltpu.VMEM)
    kernel = functools.partial(_kernel, S=S, D=D, H=H, Dh=Dh, M=M, SEG=SEG, TB=TB)
    out = pl.pallas_call(
        kernel,
        out_shape=jax.ShapeDtypeStruct((S, D), A_x.dtype),
        in_specs=[any_spec, vmem_spec] + [any_spec] * 8 + [vmem_spec],
        out_specs=any_spec,
        scratch_shapes=[
            pltpu.VMEM((S, D), BF16),
            pltpu.VMEM((3 * H, D // 2, Dh), jnp.uint32),
            pltpu.VMEM((D // LANES, H * Dh // 2, LANES), jnp.uint32),
            pltpu.VMEM((D, D), BF16),
            pltpu.VMEM((D, D), BF16),
            pltpu.VMEM((D, Fh), BF16),
            pltpu.VMEM((Fh, D), BF16),
            pltpu.VMEM((3, D * H, Dh), BF16),
            pltpu.VMEM((S + 16, D), F32),
            pltpu.VMEM((S, D), F32),
            pltpu.VMEM((S, LANES), F32),
            pltpu.VMEM((S, D), BF16),
            pltpu.SemaphoreType.DMA((S // TB,)),
            pltpu.SemaphoreType.DMA((3 * (S // TB),)),
            pltpu.SemaphoreType.DMA((4 + D // LANES,)),
        ],
        compiler_params=pltpu.CompilerParams(vmem_limit_bytes=124 * 1024 * 1024),
    )(
        A_x.reshape(S, D),
        A_mem0.reshape(M, D),
        A_Wq.reshape(D * H, Dh),
        A_Wk.reshape(D * H, Dh),
        A_Wv.reshape(D * H, Dh),
        A_Wo.reshape(H * Dh, D),
        B_w1, B_w2, B_w3, B_w4,
        gate_w.reshape(1, D),
    )
    return out.reshape(B, S, D)
```

```python
import functools
import math

import jax
import jax.numpy as jnp
from jax import lax
import jax.experimental.pallas as pl
import jax.experimental.pallas.tpu as pltpu

F32 = jnp.float32
BF16 = jnp.bfloat16
LANES = 128
LOG2E = 1.4426950408889634


def _dot(a, b):
    return lax.dot_general(a, b, (((1,), (0,)), ((), ())), preferred_element_type=F32)


def _dot_nt(a, b):
    return lax.dot_general(a, b, (((1,), (1,)), ((), ())), preferred_element_type=F32)


def _layernorm(x, eps=1e-5):
    m = jnp.mean(x, axis=-1, keepdims=True)
    xc = x - m
    v = jnp.mean(xc * xc, axis=-1, keepdims=True)
    return xc * lax.rsqrt(v + eps)


def _gelu(x):
    c = math.sqrt(2.0 / math.pi)
    return 0.5 * x * (1.0 + jnp.tanh(c * (x + 0.044715 * (x * x * x))))


def _kernel(x_hbm, mem0_ref, wq_hbm, wk_hbm, wv_hbm, wo_hbm, w1_hbm, w2_hbm, w3_hbm, w4_hbm, gw_ref,
            out_hbm,
            x_v, wqkv_v, wo_v, w1_v, w2_v, w3_v, w4_v, stage_v, h_v, bb_v, g_v, out_v, xsems, wsems,
            *, S, D, H, Dh, M, SEG, TB, NSUB):
    NSEG = S // SEG
    NT = S // TB
    DC = D // NT
    C = D // 4
    HALO = 8

    NJ = D // LANES
    NC = H // 8

    def cp_x(i):
        r0 = pl.multiple_of(i * TB, TB)
        return pltpu.make_async_copy(x_hbm.at[pl.ds(r0, TB), :], x_v.at[pl.ds(r0, TB), :], xsems.at[i])

    cp_qkv = [
        pltpu.make_async_copy(w.bitcast(jnp.uint32).at[:, pl.ds(c * 8, 8), :], stage_v.at[m * NC + c], wsems.at[4])
        for m, w in enumerate((wq_hbm, wk_hbm, wv_hbm)) for c in range(NC)]
    cp_w1 = pltpu.make_async_copy(w1_hbm, w1_v.bitcast(BF16), wsems.at[0])
    cp_w2 = pltpu.make_async_copy(w2_hbm, w2_v.bitcast(BF16), wsems.at[1])
    cp_w3 = pltpu.make_async_copy(w3_hbm, w3_v.bitcast(BF16), wsems.at[2])
    cp_w4 = pltpu.make_async_copy(w4_hbm, w4_v.bitcast(BF16), wsems.at[3])

    cp_wo = pltpu.make_async_copy(wo_hbm, wo_v.bitcast(BF16), wsems.at[5])

    cp_x(0).start()
    cp_w1.start()
    h_v[0:HALO, :] = jnp.zeros((HALO, D), F32)
    h_v[HALO + S:HALO + S + HALO, :] = jnp.zeros((HALO, D), F32)
    cp_w1.wait()
    for i in range(1, NT):
        cp_x(i).start()
    cp_w2.start()
    cp_w3.start()
    cp_w4.start()


    TS = TB // NSUB

    def b_pass1(i, _):
        cp_x(i).wait()
        xn = []
        for t in range(NSUB):
            r0 = pl.multiple_of(i * TB + t * TS, TS)
            xt = x_v[pl.ds(r0, TS), :].astype(F32)
            xn.append(_layernorm(xt).astype(BF16))
            g = jax.nn.sigmoid(jnp.sum(xt * gw_ref[...].astype(F32), axis=-1, keepdims=True))
            g_v[pl.ds(r0, TS), :] = jnp.broadcast_to(g, (TS, LANES))
        for t in range(NSUB):
            r0 = pl.multiple_of(i * TB + t * TS, TS)
            h_v[pl.ds(r0 + HALO, TS), :] = _gelu(_dot(xn[t], pltpu.bitcast(w1_v[...], BF16)))
        return 0

    lax.fori_loop(0, NT, b_pass1, 0)

    cp_w2.wait()
    cp_w3.wait()
    cp_w4.wait()
    for c in cp_qkv:
        c.start()
    cp_wo.start()

    def b_pass2(i, _):
        rows = [pl.multiple_of(i * TB + t * TS, TS) for t in range(NSUB)]
        x1 = []
        for r0 in rows:
            win = h_v[pl.ds(r0, TS + 2 * HALO), :]
            hs_in = jnp.concatenate([
                win[HALO - 1:HALO - 1 + TS, 0 * C:1 * C],
                win[HALO + 1:HALO + 1 + TS, 1 * C:2 * C],
                win[HALO - 2:HALO - 2 + TS, 2 * C:3 * C],
                win[HALO + 2:HALO + 2 + TS, 3 * C:4 * C]], axis=1).astype(BF16)
            x1.append(x_v[pl.ds(r0, TS), :].astype(F32) + _dot(hs_in, pltpu.bitcast(w2_v[...], BF16)))
        u = [_gelu(_dot(_layernorm(t).astype(BF16), pltpu.bitcast(w3_v[...], BF16))).astype(BF16) for t in x1]
        for r0, x1t, ut in zip(rows, x1, u):
            b = x1t + _dot(ut, pltpu.bitcast(w4_v[...], BF16))
            g = g_v[pl.ds(r0, TS), :]
            bb_v[pl.ds(r0, TS), :] = (1.0 - g[:, 0:1]) * b
        return 0

    lax.fori_loop(0, NT, b_pass2, 0)

    for c in cp_qkv:
        c.wait()
    stage_2d = stage_v.reshape(3 * NC, D // 2 * 8, Dh)

    def relayout(i, _):
        d0 = pl.multiple_of(i * (DC // 2), DC // 2)
        u0 = pl.multiple_of(i * (DC // 2 * 8), DC // 2 * 8)
        for m in range(3):
            for c in range(NC // 2):
                plane_e = stage_2d.at[m * NC + c, pl.ds(u0, DC // 2 * 8), :]
                plane_o = stage_2d.at[m * NC + NC // 2 + c, pl.ds(u0, DC // 2 * 8), :]
                for r in range(8):
                    even = plane_e[pl.ds(r, DC // 2, stride=8), :]
                    odd = plane_o[pl.ds(r, DC // 2, stride=8), :]
                    h = m * H + 2 * (c * 8 + r)
                    wqkv_v[h, pl.ds(d0, DC // 2), :] = (even & jnp.uint32(0xFFFF)) | (odd << 16)
                    wqkv_v[h + 1, pl.ds(d0, DC // 2), :] = (even >> 16) | (odd & jnp.uint32(0xFFFF0000))
        return 0

    lax.fori_loop(0, NT, relayout, 0)
    cp_wo.wait()

    L = M + SEG
    LP = (L + 15) // 16 * 16
    G = 4
    NG = H // G
    row = lax.broadcasted_iota(jnp.int32, (L, LP), 0)
    col = lax.broadcasted_iota(jnp.int32, (L, LP), 1)
    mask = jnp.logical_and(jnp.logical_or(row < M, row >= col), col < L)
    fill = jnp.where(col < L, -1e9 * LOG2E, -jnp.inf).astype(F32)
    qk_scale = (Dh ** -0.5) * LOG2E
    zpad = jnp.zeros((LP - L, Dh), F32)

    def cp_out(s):
        r0 = pl.multiple_of(s * SEG, SEG)
        return pltpu.make_async_copy(out_v.at[pl.ds(r0, SEG), :], out_hbm.at[pl.ds(r0, SEG), :], wsems.at[0])

    def seg_step(s, mem):
        @pl.when(s > 0)
        def _():
            cp_out(s - 1).start()

        r0 = pl.multiple_of(s * SEG, SEG)
        hcat = jnp.concatenate([mem, x_v[pl.ds(r0, SEG), :].astype(F32)], axis=0)

        def project(m, g):
            return [_dot(hcat, pltpu.bitcast(wqkv_v[m * H + g * G + t], BF16)) for t in range(G)]

        def pad_bf16(ts):
            return [jnp.concatenate([t, zpad], axis=0).astype(BF16) for t in ts]

        def softmax(sc):
            t = jnp.where(mask, sc * qk_scale, fill)
            p = jnp.exp2(t - jnp.max(t, axis=-1, keepdims=True))
            l = jnp.sum(p, axis=-1, keepdims=True)
            r = pl.reciprocal(l, approx=True)
            r = r * (2.0 - l * r)
            return p * r

        v, p, o = {}, {}, {}
        acc = [None] * NJ

        def out_proj(g, js):
            ocat = jnp.concatenate(o[g], axis=1)
            k0 = g * G * Dh // 2
            for j in js:
                w = pltpu.bitcast(wo_v[k0:k0 + G * Dh // 2, j * LANES:(j + 1) * LANES], BF16)
                part = _dot(ocat, w)
                acc[j] = part if acc[j] is None else acc[j] + part

        def attend(g):
            o[g] = [_dot(a, b) for a, b in zip(p.pop(g), v.pop(g))]

        for g in range(NG):
            q = project(0, g)
            k = pad_bf16(project(1, g))
            if g >= 1:
                attend(g - 1)
            v[g] = pad_bf16(project(2, g))
            p[g] = [softmax(_dot_nt(a, b)) for a, b in zip(q, k)]
            if g >= 2:
                out_proj(g - 2, range(NJ))
        out_proj(NG - 2, range(NJ // 2))
        attend(NG - 1)
        out_proj(NG - 2, range(NJ // 2, NJ))
        out_proj(NG - 1, range(NJ))
        res = jnp.concatenate(acc, axis=1)
        g = g_v[pl.ds(r0, SEG), :]
        out_v[pl.ds(r0, SEG), :] = (g[:, 0:1] * res[M:] + bb_v[pl.ds(r0, SEG), :]).astype(BF16)
        return res[:M]

    lax.fori_loop(0, NSEG, seg_step, mem0_ref[...].astype(F32))

    cp_out(NSEG - 1).start()
    pltpu.make_async_copy(out_v, out_hbm, wsems.at[0]).wait()


@functools.partial(jax.jit, static_argnames=("A_seg_len",))
def pallas_gated_mix__memory_aug_recurrent_mem_tr__mixer_s_mlp__prompt_kernel(
    A_x: jax.Array,
    A_mem0: jax.Array,
    A_Wq: jax.Array,
    A_Wk: jax.Array,
    A_Wv: jax.Array,
    A_Wo: jax.Array,
    A_seg_len,
    B_x: jax.Array,
    B_w1: jax.Array,
    B_w2: jax.Array,
    B_w3: jax.Array,
    B_w4: jax.Array,
    gate_w: jax.Array,
):
    del B_x
    B, S, D = A_x.shape
    assert B == 1
    _, H, Dh = A_Wq.shape
    M = A_mem0.shape[1]
    SEG = int(A_seg_len)
    Fh = B_w3.shape[1]
    TB = 256

    any_spec = pl.BlockSpec(memory_space=pl.ANY)
    vmem_spec = pl.BlockSpec(memory_space=pltpu.VMEM)
    kernel = functools.partial(_kernel, S=S, D=D, H=H, Dh=Dh, M=M, SEG=SEG, TB=TB, NSUB=2)
    out = pl.pallas_call(
        kernel,
        out_shape=jax.ShapeDtypeStruct((S, D), A_x.dtype),
        in_specs=[any_spec, vmem_spec] + [any_spec] * 8 + [vmem_spec],
        out_specs=any_spec,
        scratch_shapes=[
            pltpu.VMEM((S, D), BF16),
            pltpu.VMEM((3 * H, D // 2, Dh), jnp.uint32),
            pltpu.VMEM((H * Dh // 2, D), jnp.uint32),
            pltpu.VMEM((D // 2, D), jnp.uint32),
            pltpu.VMEM((D // 2, D), jnp.uint32),
            pltpu.VMEM((D // 2, Fh), jnp.uint32),
            pltpu.VMEM((Fh // 2, D), jnp.uint32),
            pltpu.VMEM((3 * H // 8, D // 2, 8, Dh), jnp.uint32),
            pltpu.VMEM((S + 16, D), F32),
            pltpu.VMEM((S, D), F32),
            pltpu.VMEM((S, LANES), F32),
            pltpu.VMEM((S, D), BF16),
            pltpu.SemaphoreType.DMA((S // TB,)),
            pltpu.SemaphoreType.DMA((6,)),
        ],
        compiler_params=pltpu.CompilerParams(vmem_limit_bytes=124 * 1024 * 1024),
    )(
        A_x.reshape(S, D),
        A_mem0.reshape(M, D),
        A_Wq.reshape(D // 2, 2 * H, Dh),
        A_Wk.reshape(D // 2, 2 * H, Dh),
        A_Wv.reshape(D // 2, 2 * H, Dh),
        A_Wo.reshape(H * Dh, D),
        B_w1, B_w2, B_w3, B_w4,
        gate_w.reshape(1, D),
    )
    return out.reshape(B, S, D)
```

```python
import functools
import math

import jax
import jax.numpy as jnp
from jax import lax
import jax.experimental.pallas as pl
import jax.experimental.pallas.tpu as pltpu

F32 = jnp.float32
BF16 = jnp.bfloat16
LANES = 128
LOG2E = 1.4426950408889634


def _dot(a, b):
    return lax.dot_general(a, b, (((1,), (0,)), ((), ())), preferred_element_type=F32)


def _dot_nt(a, b):
    return lax.dot_general(a, b, (((1,), (1,)), ((), ())), preferred_element_type=F32)


def _layernorm(x, eps=1e-5):
    m = jnp.mean(x, axis=-1, keepdims=True)
    xc = x - m
    v = jnp.mean(xc * xc, axis=-1, keepdims=True)
    return xc * lax.rsqrt(v + eps)


def _gelu(x):
    c = math.sqrt(2.0 / math.pi)
    return 0.5 * x * (1.0 + jnp.tanh(c * (x + 0.044715 * (x * x * x))))


def _kernel(x_hbm, mem0_ref, wq_hbm, wk_hbm, wv_hbm, wo_hbm, w1_hbm, w2_hbm, w3_hbm, w4_hbm, gw_ref,
            out_hbm,
            x_v, wqkv_v, wo_v, w1_v, w2_v, w3_v, w4_v, stage_v, h_v, bb_v, g_v, out_v, xsems, wsems,
            *, S, D, H, Dh, M, SEG, TB, NSUB):
    NSEG = S // SEG
    NT = S // TB
    DC = D // NT
    C = D // 4
    HALO = 8

    NJ = D // LANES
    NC = H // 8

    def cp_x(i):
        r0 = pl.multiple_of(i * TB, TB)
        return pltpu.make_async_copy(x_hbm.at[pl.ds(r0, TB), :], x_v.at[pl.ds(r0, TB), :], xsems.at[i])

    cp_qkv = [
        pltpu.make_async_copy(w.bitcast(jnp.uint32).at[:, pl.ds(c * 8, 8), :], stage_v.at[m * NC + c, pl.ds(0, D // 2)], wsems.at[4])
        for m, w in enumerate((wq_hbm, wk_hbm, wv_hbm)) for c in range(NC)]
    def cp_rows(src, dst_u32, sem, pieces):
        dst = dst_u32.bitcast(BF16)
        rows = src.shape[0] // pieces
        return [pltpu.make_async_copy(src.at[pl.ds(t * rows, rows), :], dst.at[pl.ds(t * rows, rows), :], sem)
                for t in range(pieces)]

    cp_w1 = cp_rows(w1_hbm, w1_v, wsems.at[0], 1)
    cp_w2 = cp_rows(w2_hbm, w2_v, wsems.at[1], 1)
    cp_w3 = cp_rows(w3_hbm, w3_v, wsems.at[2], 1)
    cp_w4 = cp_rows(w4_hbm, w4_v, wsems.at[3], 1)
    cp_wo = cp_rows(wo_hbm, wo_v, wsems.at[5], 1)

    cp_x(0).start()
    for c in cp_w1:
        c.start()
    for i in range(1, NT):
        cp_x(i).start()
    for c in cp_w2 + cp_w3 + cp_w4 + cp_qkv + cp_wo:
        c.start()
    h_v[0:HALO, :] = jnp.zeros((HALO, D), F32)
    h_v[HALO + S:HALO + S + HALO, :] = jnp.zeros((HALO, D), F32)

    TS = TB // NSUB

    gw = gw_ref[...].astype(F32).reshape(1, D)

    def norm_and_gate(r0):
        xt = x_v[pl.ds(r0, TS), :].astype(F32)
        g = jax.nn.sigmoid(jnp.sum(xt * gw, axis=-1, keepdims=True))
        g_v[pl.ds(r0, TS), :] = jnp.broadcast_to(g, (TS, LANES))
        return _layernorm(xt).astype(BF16)

    def b_pass1(i, xn0):
        @pl.when(i + 1 < NT)
        def _():
            cp_x(i + 1).wait()

        rows = [pl.multiple_of(i * TB + t * TS, TS) for t in range(NSUB)]
        xn = [xn0] + [norm_and_gate(r0) for r0 in rows[1:]]
        for r0, t in zip(rows, xn):
            h_v[pl.ds(r0 + HALO, TS), :] = _gelu(_dot(t, pltpu.bitcast(w1_v[...], BF16)))
        return norm_and_gate(pl.multiple_of(jnp.minimum(i + 1, NT - 1) * TB, TB))

    cp_x(0).wait()
    xn_first = norm_and_gate(0)
    for c in cp_w1:
        c.wait()

    lax.fori_loop(0, NT, b_pass1, xn_first)

    for c in cp_w2 + cp_w3 + cp_w4:
        c.wait()

    def b_pass2(i, _):
        rows = [pl.multiple_of(i * TB + t * TS, TS) for t in range(NSUB)]
        x1 = []
        for r0 in rows:
            win = h_v[pl.ds(r0, TS + 2 * HALO), :]
            hs_in = jnp.concatenate([
                win[HALO - 1:HALO - 1 + TS, 0 * C:1 * C],
                win[HALO + 1:HALO + 1 + TS, 1 * C:2 * C],
                win[HALO - 2:HALO - 2 + TS, 2 * C:3 * C],
                win[HALO + 2:HALO + 2 + TS, 3 * C:4 * C]], axis=1).astype(BF16)
            x1.append(x_v[pl.ds(r0, TS), :].astype(F32) + _dot(hs_in, pltpu.bitcast(w2_v[...], BF16)))
        u = [_gelu(_dot(_layernorm(t).astype(BF16), pltpu.bitcast(w3_v[...], BF16))).astype(BF16) for t in x1]
        for r0, x1t, ut in zip(rows, x1, u):
            b = x1t + _dot(ut, pltpu.bitcast(w4_v[...], BF16))
            g = g_v[pl.ds(r0, TS), :]
            bb_v[pl.ds(r0, TS), :] = (1.0 - g[:, 0:1]) * b
        return 0

    lax.fori_loop(0, NT, b_pass2, 0)

    for c in cp_qkv + cp_wo:
        c.wait()

    L = M + SEG
    LP = (L + 15) // 16 * 16
    G = 4
    NG = H // G
    row = lax.broadcasted_iota(jnp.int32, (L, LP), 0)
    col = lax.broadcasted_iota(jnp.int32, (L, LP), 1)
    mask = jnp.logical_and(jnp.logical_or(row < M, row >= col), col < L)
    fill = jnp.where(col < L, -1e9 * LOG2E, -jnp.inf).astype(F32)
    qk_scale = (Dh ** -0.5) * LOG2E
    zpad = jnp.zeros((LP - L, Dh), F32)

    def cp_out(s):
        r0 = pl.multiple_of(s * SEG, SEG)
        return pltpu.make_async_copy(out_v.at[pl.ds(r0, SEG), :], out_hbm.at[pl.ds(r0, SEG), :], wsems.at[0])

    stage_2d = stage_v.reshape(3 * NC, (D // 2 + 1) * 8, Dh)

    def build_slabs(m, g):
        slabs = []
        for h in range(g * G, (g + 1) * G, 2):
            c, r = divmod(h // 2, 8)
            even = stage_2d[m * NC + c, pl.ds(r, D // 2, stride=8), :]
            odd = stage_2d[m * NC + NC // 2 + c, pl.ds(r, D // 2, stride=8), :]
            slabs.append((even & jnp.uint32(0xFFFF)) | (odd << 16))
            slabs.append((even >> 16) | (odd & jnp.uint32(0xFFFF0000)))
        for t, w in enumerate(slabs):
            wqkv_v[m * H + g * G + t] = w
        return slabs

    def load_slabs(m, g):
        return [wqkv_v[m * H + g * G + t] for t in range(G)]

    def seg_step(s, mem, get_slabs):
        r0 = s * SEG if isinstance(s, int) else pl.multiple_of(s * SEG, SEG)
        hcat = jnp.concatenate([mem, x_v[pl.ds(r0, SEG), :].astype(F32)], axis=0)

        def project(m, g):
            return [_dot(hcat, pltpu.bitcast(w, BF16)) for w in get_slabs(m, g)]

        def pad_bf16(ts):
            return [jnp.concatenate([t, zpad], axis=0).astype(BF16) for t in ts]

        def softmax(sc):
            t = jnp.where(mask, sc * qk_scale, fill)
            p = jnp.exp2(t - jnp.max(t, axis=-1, keepdims=True))
            l = jnp.sum(p, axis=-1, keepdims=True)
            r = pl.reciprocal(l, approx=True)
            r = r * (2.0 - l * r)
            return p * r

        v, p, o = {}, {}, {}
        acc = [None] * NJ

        def out_proj(g, js):
            ocat = jnp.concatenate(o[g], axis=1)
            k0 = g * G * Dh // 2
            for j in js:
                w = pltpu.bitcast(wo_v[k0:k0 + G * Dh // 2, j * LANES:(j + 1) * LANES], BF16)
                part = _dot(ocat, w)
                acc[j] = part if acc[j] is None else acc[j] + part

        def attend(g):
            o[g] = [_dot(a, b) for a, b in zip(p.pop(g), v.pop(g))]

        for g in range(NG):
            q = project(0, g)
            k = pad_bf16(project(1, g))
            if g >= 1:
                attend(g - 1)
            v[g] = pad_bf16(project(2, g))
            p[g] = [softmax(_dot_nt(a, b)) for a, b in zip(q, k)]
            if g >= 2:
                out_proj(g - 2, range(NJ))
        out_proj(NG - 2, range(NJ // 2))
        attend(NG - 1)
        out_proj(NG - 2, range(NJ // 2, NJ))
        out_proj(NG - 1, range(NJ))
        res = jnp.concatenate(acc, axis=1)
        g = g_v[pl.ds(r0, SEG), :]
        out_v[pl.ds(r0, SEG), :] = (g[:, 0:1] * res[M:] + bb_v[pl.ds(r0, SEG), :]).astype(BF16)
        return res[:M]

    def later_step(s, mem):
        cp_out(s - 1).start()
        return seg_step(s, mem, load_slabs)

    mem1 = seg_step(0, mem0_ref[...].astype(F32), build_slabs)
    lax.fori_loop(1, NSEG, later_step, mem1)

    cp_out(NSEG - 1).start()
    pltpu.make_async_copy(out_v, out_hbm, wsems.at[0]).wait()


@functools.partial(jax.jit, static_argnames=("A_seg_len",))
def pallas_gated_mix__memory_aug_recurrent_mem_tr__mixer_s_mlp__prompt_kernel(
    A_x: jax.Array,
    A_mem0: jax.Array,
    A_Wq: jax.Array,
    A_Wk: jax.Array,
    A_Wv: jax.Array,
    A_Wo: jax.Array,
    A_seg_len,
    B_x: jax.Array,
    B_w1: jax.Array,
    B_w2: jax.Array,
    B_w3: jax.Array,
    B_w4: jax.Array,
    gate_w: jax.Array,
):
    del B_x
    B, S, D = A_x.shape
    assert B == 1
    _, H, Dh = A_Wq.shape
    M = A_mem0.shape[1]
    SEG = int(A_seg_len)
    Fh = B_w3.shape[1]
    TB = 256

    any_spec = pl.BlockSpec(memory_space=pl.ANY)
    vmem_spec = pl.BlockSpec(memory_space=pltpu.VMEM)
    kernel = functools.partial(_kernel, S=S, D=D, H=H, Dh=Dh, M=M, SEG=SEG, TB=TB, NSUB=2)
    out = pl.pallas_call(
        kernel,
        out_shape=jax.ShapeDtypeStruct((S, D), A_x.dtype),
        in_specs=[any_spec, vmem_spec] + [any_spec] * 8 + [vmem_spec],
        out_specs=any_spec,
        scratch_shapes=[
            pltpu.VMEM((S, D), BF16),
            pltpu.VMEM((3 * H, D // 2, Dh), jnp.uint32),
            pltpu.VMEM((H * Dh // 2, D), jnp.uint32),
            pltpu.VMEM((D // 2, D), jnp.uint32),
            pltpu.VMEM((D // 2, D), jnp.uint32),
            pltpu.VMEM((D // 2, Fh), jnp.uint32),
            pltpu.VMEM((Fh // 2, D), jnp.uint32),
            pltpu.VMEM((3 * H // 8, D // 2 + 1, 8, Dh), jnp.uint32),
            pltpu.VMEM((S + 16, D), F32),
            pltpu.VMEM((S, D), F32),
            pltpu.VMEM((S, LANES), F32),
            pltpu.VMEM((S, D), BF16),
            pltpu.SemaphoreType.DMA((S // TB,)),
            pltpu.SemaphoreType.DMA((6,)),
        ],
        compiler_params=pltpu.CompilerParams(vmem_limit_bytes=124 * 1024 * 1024),
    )(
        A_x.reshape(S, D),
        A_mem0.reshape(M, D),
        A_Wq.reshape(D // 2, 2 * H, Dh),
        A_Wk.reshape(D // 2, 2 * H, Dh),
        A_Wv.reshape(D // 2, 2 * H, Dh),
        A_Wo.reshape(H * Dh, D),
        B_w1, B_w2, B_w3, B_w4,
        gate_w,
    )
    return out.reshape(B, S, D)
```

```python
import functools
import math

import jax
import jax.numpy as jnp
from jax import lax
import jax.experimental.pallas as pl
import jax.experimental.pallas.tpu as pltpu

F32 = jnp.float32
BF16 = jnp.bfloat16
LANES = 128
LOG2E = 1.4426950408889634


def _dot(a, b):
    return lax.dot_general(a, b, (((1,), (0,)), ((), ())), preferred_element_type=F32)


def _dot_nt(a, b):
    return lax.dot_general(a, b, (((1,), (1,)), ((), ())), preferred_element_type=F32)


def _layernorm(x, eps=1e-5):
    m = jnp.mean(x, axis=-1, keepdims=True)
    xc = x - m
    v = jnp.mean(xc * xc, axis=-1, keepdims=True)
    return xc * lax.rsqrt(v + eps)


def _gelu(x):
    c = math.sqrt(2.0 / math.pi)
    return 0.5 * x * (1.0 + jnp.tanh(c * (x + 0.044715 * (x * x * x))))


def _kernel(x_hbm, mem0_ref, wq_hbm, wk_hbm, wv_hbm, wo_hbm, w1_hbm, w2_hbm, w3_hbm, w4_hbm, gw_ref,
            out_hbm,
            x_v, wqkv_v, wo_v, w1_v, w2_v, w3_v, w4_v, stage_v, h_v, bb_v, g_v, out_v, xsems, wsems,
            *, S, D, H, Dh, M, SEG, TB, NSUB):
    NSEG = S // SEG
    NT = S // TB
    DC = D // NT
    C = D // 4
    HALO = 8

    NJ = D // LANES
    NC = H // 8

    def cp_x(i):
        r0 = pl.multiple_of(i * TB, TB)
        return pltpu.make_async_copy(x_hbm.at[pl.ds(r0, TB), :], x_v.at[pl.ds(r0, TB), :], xsems.at[i])

    cp_qkv = [
        pltpu.make_async_copy(w.bitcast(jnp.uint32).at[:, pl.ds(c * 8, 8), :], stage_v.at[m * NC + c, pl.ds(0, D // 2)], wsems.at[4])
        for m, w in enumerate((wq_hbm, wk_hbm, wv_hbm)) for c in range(NC)]
    def cp_rows(src, dst_u32, sem, pieces):
        dst = dst_u32.bitcast(BF16)
        rows = src.shape[0] // pieces
        return [pltpu.make_async_copy(src.at[pl.ds(t * rows, rows), :], dst.at[pl.ds(t * rows, rows), :], sem)
                for t in range(pieces)]

    cp_w1 = cp_rows(w1_hbm, w1_v, wsems.at[0], 1)
    cp_w2 = cp_rows(w2_hbm, w2_v, wsems.at[1], 1)
    cp_w3 = cp_rows(w3_hbm, w3_v, wsems.at[2], 1)
    cp_w4 = cp_rows(w4_hbm, w4_v, wsems.at[3], 1)
    cp_wo = cp_rows(wo_hbm, wo_v, wsems.at[5], 1)

    cp_x(0).start()
    for c in cp_w1:
        c.start()
    for i in range(1, NT):
        cp_x(i).start()
    for c in cp_w2 + cp_w3 + cp_w4 + cp_qkv + cp_wo:
        c.start()
    h_v[0:HALO, :] = jnp.zeros((HALO, D), F32)
    h_v[HALO + S:HALO + S + HALO, :] = jnp.zeros((HALO, D), F32)

    TS = TB // NSUB

    gw = gw_ref[...].astype(F32).reshape(1, D)

    def norm_and_gate(r0):
        xt = x_v[pl.ds(r0, TS), :].astype(F32)
        g = jax.nn.sigmoid(jnp.sum(xt * gw, axis=-1, keepdims=True))
        g_v[pl.ds(r0, TS), :] = jnp.broadcast_to(g, (TS, LANES))
        return _layernorm(xt).astype(BF16)

    def b_pass1(i, xn0):
        @pl.when(i + 1 < NT)
        def _():
            cp_x(i + 1).wait()

        rows = [pl.multiple_of(i * TB + t * TS, TS) for t in range(NSUB)]
        xn = [xn0] + [norm_and_gate(r0) for r0 in rows[1:]]
        for r0, t in zip(rows, xn):
            h_v[pl.ds(r0 + HALO, TS), :] = _gelu(_dot(t, pltpu.bitcast(w1_v[...], BF16)))
        return norm_and_gate(pl.multiple_of(jnp.minimum(i + 1, NT - 1) * TB, TB))

    cp_x(0).wait()
    xn_first = norm_and_gate(0)
    for c in cp_w1:
        c.wait()

    lax.fori_loop(0, NT, b_pass1, xn_first)

    for c in cp_w2 + cp_w3 + cp_w4:
        c.wait()

    def b_pass2(i, _):
        rows = [pl.multiple_of(i * TB + t * TS, TS) for t in range(NSUB)]
        x1 = []
        for r0 in rows:
            win = h_v[pl.ds(r0, TS + 2 * HALO), :]
            hs_in = jnp.concatenate([
                win[HALO - 1:HALO - 1 + TS, 0 * C:1 * C],
                win[HALO + 1:HALO + 1 + TS, 1 * C:2 * C],
                win[HALO - 2:HALO - 2 + TS, 2 * C:3 * C],
                win[HALO + 2:HALO + 2 + TS, 3 * C:4 * C]], axis=1).astype(BF16)
            x1.append(x_v[pl.ds(r0, TS), :].astype(F32) + _dot(hs_in, pltpu.bitcast(w2_v[...], BF16)))
        u = [_gelu(_dot(_layernorm(t).astype(BF16), pltpu.bitcast(w3_v[...], BF16))).astype(BF16) for t in x1]
        for r0, x1t, ut in zip(rows, x1, u):
            b = x1t + _dot(ut, pltpu.bitcast(w4_v[...], BF16))
            g = g_v[pl.ds(r0, TS), :]
            bb_v[pl.ds(r0, TS), :] = (1.0 - g[:, 0:1]) * b
        return 0

    lax.fori_loop(0, NT, b_pass2, 0)

    for c in cp_qkv + cp_wo:
        c.wait()

    L = M + SEG
    LP = (L + 15) // 16 * 16
    G = 4
    NG = H // G
    row = lax.broadcasted_iota(jnp.int32, (L, LP), 0)
    col = lax.broadcasted_iota(jnp.int32, (L, LP), 1)
    mask = jnp.logical_and(jnp.logical_or(row < M, row >= col), col < L)
    fill = jnp.where(col < L, -1e9 * LOG2E, -jnp.inf).astype(F32)
    qk_scale = (Dh ** -0.5) * LOG2E
    zpad = jnp.zeros((LP - L, Dh), F32)

    def cp_out(s):
        r0 = pl.multiple_of(s * SEG, SEG)
        return pltpu.make_async_copy(out_v.at[pl.ds(r0, SEG), :], out_hbm.at[pl.ds(r0, SEG), :], wsems.at[0])

    stage_2d = stage_v.reshape(3 * NC, (D // 2 + 1) * 8, Dh)

    def project_building(hcat, m, g):
        KW = LANES // 2
        acc = [None] * G
        for kt in range(D // LANES):
            lhs = hcat[:, kt * LANES:(kt + 1) * LANES]
            for t in range(0, G, 2):
                h = g * G + t
                c, r = divmod(h // 2, 8)
                rows = pl.ds(kt * KW * 8 + r, KW, stride=8)
                even = stage_2d[m * NC + c, rows, :]
                odd = stage_2d[m * NC + NC // 2 + c, rows, :]
                pair = ((even & jnp.uint32(0xFFFF)) | (odd << 16), (even >> 16) | (odd & jnp.uint32(0xFFFF0000)))
                for n, w in enumerate(pair):
                    wqkv_v[m * H + h + n, kt * KW:(kt + 1) * KW, :] = w
                    part = _dot(lhs, pltpu.bitcast(w, BF16))
                    acc[t + n] = part if kt == 0 else acc[t + n] + part
        return acc

    def project_stored(hcat, m, g):
        return [_dot(hcat, pltpu.bitcast(wqkv_v[m * H + g * G + t], BF16)) for t in range(G)]

    def seg_step(s, mem, project_fn):
        r0 = s * SEG if isinstance(s, int) else pl.multiple_of(s * SEG, SEG)
        hcat = jnp.concatenate([mem, x_v[pl.ds(r0, SEG), :].astype(F32)], axis=0)

        project = functools.partial(project_fn, hcat)

        def pad_bf16(ts):
            return [jnp.concatenate([t, zpad], axis=0).astype(BF16) for t in ts]

        def softmax(sc):
            t = jnp.where(mask, sc * qk_scale, fill)
            p = jnp.exp2(t - jnp.max(t, axis=-1, keepdims=True))
            l = jnp.sum(p, axis=-1, keepdims=True)
            r = pl.reciprocal(l, approx=True)
            r = r * (2.0 - l * r)
            return p * r

        v, p, o = {}, {}, {}
        acc = [None] * NJ

        def out_proj(g, js):
            ocat = jnp.concatenate(o[g], axis=1)
            k0 = g * G * Dh // 2
            for j in js:
                w = pltpu.bitcast(wo_v[k0:k0 + G * Dh // 2, j * LANES:(j + 1) * LANES], BF16)
                part = _dot(ocat, w)
                acc[j] = part if acc[j] is None else acc[j] + part

        def attend(g):
            o[g] = [_dot(a, b) for a, b in zip(p.pop(g), v.pop(g))]

        for g in range(NG):
            q = project(0, g)
            k = pad_bf16(project(1, g))
            if g >= 1:
                attend(g - 1)
            v[g] = pad_bf16(project(2, g))
            p[g] = [softmax(_dot_nt(a, b)) for a, b in zip(q, k)]
            if g >= 2:
                out_proj(g - 2, range(NJ))
        out_proj(NG - 2, range(NJ // 2))
        attend(NG - 1)
        out_proj(NG - 2, range(NJ // 2, NJ))
        out_proj(NG - 1, range(NJ))
        res = jnp.concatenate(acc, axis=1)
        g = g_v[pl.ds(r0, SEG), :]
        out_v[pl.ds(r0, SEG), :] = (g[:, 0:1] * res[M:] + bb_v[pl.ds(r0, SEG), :]).astype(BF16)
        return res[:M]

    def later_step(s, mem):
        cp_out(s - 1).start()
        return seg_step(s, mem, project_stored)

    mem1 = seg_step(0, mem0_ref[...].astype(F32), project_building)
    lax.fori_loop(1, NSEG, later_step, mem1)

    cp_out(NSEG - 1).start()
    pltpu.make_async_copy(out_v, out_hbm, wsems.at[0]).wait()


@functools.partial(jax.jit, static_argnames=("A_seg_len",))
def pallas_gated_mix__memory_aug_recurrent_mem_tr__mixer_s_mlp__prompt_kernel(
    A_x: jax.Array,
    A_mem0: jax.Array,
    A_Wq: jax.Array,
    A_Wk: jax.Array,
    A_Wv: jax.Array,
    A_Wo: jax.Array,
    A_seg_len,
    B_x: jax.Array,
    B_w1: jax.Array,
    B_w2: jax.Array,
    B_w3: jax.Array,
    B_w4: jax.Array,
    gate_w: jax.Array,
):
    del B_x
    B, S, D = A_x.shape
    assert B == 1
    _, H, Dh = A_Wq.shape
    M = A_mem0.shape[1]
    SEG = int(A_seg_len)
    Fh = B_w3.shape[1]
    TB = 256

    any_spec = pl.BlockSpec(memory_space=pl.ANY)
    vmem_spec = pl.BlockSpec(memory_space=pltpu.VMEM)
    kernel = functools.partial(_kernel, S=S, D=D, H=H, Dh=Dh, M=M, SEG=SEG, TB=TB, NSUB=2)
    out = pl.pallas_call(
        kernel,
        out_shape=jax.ShapeDtypeStruct((S, D), A_x.dtype),
        in_specs=[any_spec, vmem_spec] + [any_spec] * 8 + [vmem_spec],
        out_specs=any_spec,
        scratch_shapes=[
            pltpu.VMEM((S, D), BF16),
            pltpu.VMEM((3 * H, D // 2, Dh), jnp.uint32),
            pltpu.VMEM((H * Dh // 2, D), jnp.uint32),
            pltpu.VMEM((D // 2, D), jnp.uint32),
            pltpu.VMEM((D // 2, D), jnp.uint32),
            pltpu.VMEM((D // 2, Fh), jnp.uint32),
            pltpu.VMEM((Fh // 2, D), jnp.uint32),
            pltpu.VMEM((3 * H // 8, D // 2 + 1, 8, Dh), jnp.uint32),
            pltpu.VMEM((S + 16, D), F32),
            pltpu.VMEM((S, D), F32),
            pltpu.VMEM((S, LANES), F32),
            pltpu.VMEM((S, D), BF16),
            pltpu.SemaphoreType.DMA((S // TB,)),
            pltpu.SemaphoreType.DMA((6,)),
        ],
        compiler_params=pltpu.CompilerParams(vmem_limit_bytes=124 * 1024 * 1024),
    )(
        A_x.reshape(S, D),
        A_mem0.reshape(M, D),
        A_Wq.reshape(D // 2, 2 * H, Dh),
        A_Wk.reshape(D // 2, 2 * H, Dh),
        A_Wv.reshape(D // 2, 2 * H, Dh),
        A_Wo.reshape(H * Dh, D),
        B_w1, B_w2, B_w3, B_w4,
        gate_w,
    )
    return out.reshape(B, S, D)
```

```python
import functools
import math

import jax
import jax.numpy as jnp
from jax import lax
import jax.experimental.pallas as pl
import jax.experimental.pallas.tpu as pltpu

F32 = jnp.float32
BF16 = jnp.bfloat16
LANES = 128
LOG2E = 1.4426950408889634


def _dot(a, b):
    return lax.dot_general(a, b, (((1,), (0,)), ((), ())), preferred_element_type=F32)


def _dot_nt(a, b):
    return lax.dot_general(a, b, (((1,), (1,)), ((), ())), preferred_element_type=F32)


def _layernorm(x, eps=1e-5):
    m = jnp.mean(x, axis=-1, keepdims=True)
    xc = x - m
    v = jnp.mean(xc * xc, axis=-1, keepdims=True)
    return xc * lax.rsqrt(v + eps)


def _gelu(x):
    c = math.sqrt(2.0 / math.pi)
    return 0.5 * x * (1.0 + jnp.tanh(c * (x + 0.044715 * (x * x * x))))


def _kernel(x_hbm, mem0_ref, wq_hbm, wk_hbm, wv_hbm, wo_hbm, w1_hbm, w2_hbm, w3_hbm, w4_hbm, gw_ref,
            out_hbm,
            x_v, wqkv_v, wo_v, w1_v, w2_v, w3_v, w4_v, stage_v, h_v, bb_v, g_v, out_v, xsems, wsems,
            *, S, D, H, Dh, M, SEG, TB, NSUB):
    NSEG = S // SEG
    NT = S // TB
    DC = D // NT
    C = D // 4
    HALO = 8

    NJ = D // LANES
    NC = H // 8

    def cp_x(i):
        r0 = pl.multiple_of(i * TB, TB)
        return pltpu.make_async_copy(x_hbm.at[pl.ds(r0, TB), :], x_v.at[pl.ds(r0, TB), :], xsems.at[i])

    def plane(m, parity, c):
        return (m * 2 + parity) * NC + c

    cp_qkv = [
        pltpu.make_async_copy(
            w.bitcast(jnp.uint32).at[:, pl.ds((parity + 2 * half) * (H // 2) + 4 * c, 4), :],
            stage_v.at[plane(m, parity, c), pl.ds(0, D // 4), pl.ds(4 * half, 4), :], wsems.at[4])
        for m, w in enumerate((wq_hbm, wk_hbm, wv_hbm))
        for parity in range(2) for c in range(NC) for half in range(2)]

    def cp_rows(src, dst_u32, sem, pieces):
        dst = dst_u32.bitcast(BF16)
        rows = src.shape[0] // pieces
        return [pltpu.make_async_copy(src.at[pl.ds(t * rows, rows), :], dst.at[pl.ds(t * rows, rows), :], sem)
                for t in range(pieces)]

    cp_w1 = cp_rows(w1_hbm, w1_v, wsems.at[0], 1)
    cp_w2 = cp_rows(w2_hbm, w2_v, wsems.at[1], 1)
    cp_w3 = cp_rows(w3_hbm, w3_v, wsems.at[2], 1)
    cp_w4 = cp_rows(w4_hbm, w4_v, wsems.at[3], 1)
    cp_wo = cp_rows(wo_hbm, wo_v, wsems.at[5], 1)

    cp_x(0).start()
    for c in cp_w1:
        c.start()
    for i in range(1, NT):
        cp_x(i).start()
    for c in cp_w2 + cp_w3 + cp_w4:
        c.start()
    h_v[0:HALO, :] = jnp.zeros((HALO, D), F32)
    h_v[HALO + S:HALO + S + HALO, :] = jnp.zeros((HALO, D), F32)

    TS = TB // NSUB

    gw = gw_ref[...].astype(F32).reshape(1, D)

    def norm_and_gate(r0):
        xt = x_v[pl.ds(r0, TS), :].astype(F32)
        g = jax.nn.sigmoid(jnp.sum(xt * gw, axis=-1, keepdims=True))
        g_v[pl.ds(r0, TS), :] = jnp.broadcast_to(g, (TS, LANES))
        return _layernorm(xt).astype(BF16)

    def b_pass1(i, xn0):
        @pl.when(i + 1 < NT)
        def _():
            cp_x(i + 1).wait()

        rows = [pl.multiple_of(i * TB + t * TS, TS) for t in range(NSUB)]
        xn = [xn0] + [norm_and_gate(r0) for r0 in rows[1:]]
        for r0, t in zip(rows, xn):
            h_v[pl.ds(r0 + HALO, TS), :] = _gelu(_dot(t, pltpu.bitcast(w1_v[...], BF16)))
        return norm_and_gate(pl.multiple_of(jnp.minimum(i + 1, NT - 1) * TB, TB))

    cp_x(0).wait()
    xn_first = norm_and_gate(0)
    for c in cp_w1:
        c.wait()

    lax.fori_loop(0, NT, b_pass1, xn_first)

    for c in cp_qkv + cp_wo:
        c.start()
    for c in cp_w2 + cp_w3 + cp_w4:
        c.wait()

    def b_pass2(i, _):
        rows = [pl.multiple_of(i * TB + t * TS, TS) for t in range(NSUB)]
        x1 = []
        for r0 in rows:
            win = h_v[pl.ds(r0, TS + 2 * HALO), :]
            hs_in = jnp.concatenate([
                win[HALO - 1:HALO - 1 + TS, 0 * C:1 * C],
                win[HALO + 1:HALO + 1 + TS, 1 * C:2 * C],
                win[HALO - 2:HALO - 2 + TS, 2 * C:3 * C],
                win[HALO + 2:HALO + 2 + TS, 3 * C:4 * C]], axis=1).astype(BF16)
            x1.append(x_v[pl.ds(r0, TS), :].astype(F32) + _dot(hs_in, pltpu.bitcast(w2_v[...], BF16)))
        u = [_gelu(_dot(_layernorm(t).astype(BF16), pltpu.bitcast(w3_v[...], BF16))).astype(BF16) for t in x1]
        for r0, x1t, ut in zip(rows, x1, u):
            b = x1t + _dot(ut, pltpu.bitcast(w4_v[...], BF16))
            g = g_v[pl.ds(r0, TS), :]
            bb_v[pl.ds(r0, TS), :] = (1.0 - g[:, 0:1]) * b
        return 0

    lax.fori_loop(0, NT, b_pass2, 0)

    for c in cp_qkv + cp_wo:
        c.wait()

    L = M + SEG
    LP = (L + 15) // 16 * 16
    G = 4
    NG = H // G
    row = lax.broadcasted_iota(jnp.int32, (L, LP), 0)
    col = lax.broadcasted_iota(jnp.int32, (L, LP), 1)
    mask = jnp.logical_and(jnp.logical_or(row < M, row >= col), col < L)
    fill = jnp.where(col < L, -1e9 * LOG2E, -jnp.inf).astype(F32)
    qk_scale = (Dh ** -0.5) * LOG2E
    zpad = jnp.zeros((LP - L, Dh), F32)

    def cp_out(s):
        r0 = pl.multiple_of(s * SEG, SEG)
        return pltpu.make_async_copy(out_v.at[pl.ds(r0, SEG), :], out_hbm.at[pl.ds(r0, SEG), :], wsems.at[0])

    stage_2d = stage_v.reshape(6 * NC, (D // 4 + 1) * 8, Dh)

    def project_building(hcat, m, g):
        KW = LANES // 2
        acc = [None] * G
        for kt in range(D // LANES):
            lhs = hcat[:, kt * LANES:(kt + 1) * LANES]
            for t in range(0, G, 2):
                h = g * G + t
                c, r = divmod(h // 2, 4)
                rows = pl.ds(kt * KW * 4 + r, KW, stride=4)
                even = stage_2d[plane(m, 0, c), rows, :]
                odd = stage_2d[plane(m, 1, c), rows, :]
                pair = ((even & jnp.uint32(0xFFFF)) | (odd << 16), (even >> 16) | (odd & jnp.uint32(0xFFFF0000)))
                for n, w in enumerate(pair):
                    wqkv_v[m * H + h + n, kt * KW:(kt + 1) * KW, :] = w
                    part = _dot(lhs, pltpu.bitcast(w, BF16))
                    acc[t + n] = part if kt == 0 else acc[t + n] + part
        return acc

    def project_stored(hcat, m, g):
        return [_dot(hcat, pltpu.bitcast(wqkv_v[m * H + g * G + t], BF16)) for t in range(G)]

    def seg_step(s, mem, project_fn):
        r0 = s * SEG if isinstance(s, int) else pl.multiple_of(s * SEG, SEG)
        hcat = jnp.concatenate([mem, x_v[pl.ds(r0, SEG), :].astype(F32)], axis=0)

        project = functools.partial(project_fn, hcat)

        def pad_bf16(ts):
            return [jnp.concatenate([t, zpad], axis=0).astype(BF16) for t in ts]

        def softmax(sc):
            t = jnp.where(mask, sc * qk_scale, fill)
            p = jnp.exp2(t - jnp.max(t, axis=-1, keepdims=True))
            l = jnp.sum(p, axis=-1, keepdims=True)
            r = pl.reciprocal(l, approx=True)
            r = r * (2.0 - l * r)
            return p * r

        v, p, o = {}, {}, {}
        acc = [None] * NJ

        def out_proj(g, js):
            ocat = jnp.concatenate(o[g], axis=1)
            k0 = g * G * Dh // 2
            for j in js:
                w = pltpu.bitcast(wo_v[k0:k0 + G * Dh // 2, j * LANES:(j + 1) * LANES], BF16)
                part = _dot(ocat, w)
                acc[j] = part if acc[j] is None else acc[j] + part

        def attend(g):
            o[g] = [_dot(a, b) for a, b in zip(p.pop(g), v.pop(g))]

        for g in range(NG):
            q = project(0, g)
            k = pad_bf16(project(1, g))
            if g >= 1:
                attend(g - 1)
            v[g] = pad_bf16(project(2, g))
            p[g] = [softmax(_dot_nt(a, b)) for a, b in zip(q, k)]
            if g >= 2:
                out_proj(g - 2, range(NJ))
        out_proj(NG - 2, range(NJ // 2))
        attend(NG - 1)
        out_proj(NG - 2, range(NJ // 2, NJ))
        out_proj(NG - 1, range(NJ))
        res = jnp.concatenate(acc, axis=1)
        g = g_v[pl.ds(r0, SEG), :]
        out_v[pl.ds(r0, SEG), :] = (g[:, 0:1] * res[M:] + bb_v[pl.ds(r0, SEG), :]).astype(BF16)
        return res[:M]

    def later_step(s, mem):
        cp_out(s - 1).start()
        return seg_step(s, mem, project_stored)

    mem1 = seg_step(0, mem0_ref[...].astype(F32), project_building)
    lax.fori_loop(1, NSEG, later_step, mem1)

    cp_out(NSEG - 1).start()
    pltpu.make_async_copy(out_v, out_hbm, wsems.at[0]).wait()


@functools.partial(jax.jit, static_argnames=("A_seg_len",))
def pallas_gated_mix__memory_aug_recurrent_mem_tr__mixer_s_mlp__prompt_kernel(
    A_x: jax.Array,
    A_mem0: jax.Array,
    A_Wq: jax.Array,
    A_Wk: jax.Array,
    A_Wv: jax.Array,
    A_Wo: jax.Array,
    A_seg_len,
    B_x: jax.Array,
    B_w1: jax.Array,
    B_w2: jax.Array,
    B_w3: jax.Array,
    B_w4: jax.Array,
    gate_w: jax.Array,
):
    del B_x
    B, S, D = A_x.shape
    assert B == 1
    _, H, Dh = A_Wq.shape
    M = A_mem0.shape[1]
    SEG = int(A_seg_len)
    Fh = B_w3.shape[1]
    TB = 256

    any_spec = pl.BlockSpec(memory_space=pl.ANY)
    vmem_spec = pl.BlockSpec(memory_space=pltpu.VMEM)
    kernel = functools.partial(_kernel, S=S, D=D, H=H, Dh=Dh, M=M, SEG=SEG, TB=TB, NSUB=2)
    out = pl.pallas_call(
        kernel,
        out_shape=jax.ShapeDtypeStruct((S, D), A_x.dtype),
        in_specs=[any_spec, vmem_spec] + [any_spec] * 8 + [vmem_spec],
        out_specs=any_spec,
        scratch_shapes=[
            pltpu.VMEM((S, D), BF16),
            pltpu.VMEM((3 * H, D // 2, Dh), jnp.uint32),
            pltpu.VMEM((H * Dh // 2, D), jnp.uint32),
            pltpu.VMEM((D // 2, D), jnp.uint32),
            pltpu.VMEM((D // 2, D), jnp.uint32),
            pltpu.VMEM((D // 2, Fh), jnp.uint32),
            pltpu.VMEM((Fh // 2, D), jnp.uint32),
            pltpu.VMEM((6 * H // 8, D // 4 + 1, 8, Dh), jnp.uint32),
            pltpu.VMEM((S + 16, D), F32),
            pltpu.VMEM((S, D), F32),
            pltpu.VMEM((S, LANES), F32),
            pltpu.VMEM((S, D), BF16),
            pltpu.SemaphoreType.DMA((S // TB,)),
            pltpu.SemaphoreType.DMA((6,)),
        ],
        compiler_params=pltpu.CompilerParams(vmem_limit_bytes=124 * 1024 * 1024),
    )(
        A_x.reshape(S, D),
        A_mem0.reshape(M, D),
        A_Wq.reshape(D // 4, 4 * H, Dh),
        A_Wk.reshape(D // 4, 4 * H, Dh),
        A_Wv.reshape(D // 4, 4 * H, Dh),
        A_Wo.reshape(H * Dh, D),
        B_w1, B_w2, B_w3, B_w4,
        gate_w,
    )
    return out.reshape(B, S, D)
```

```python
import functools
import math

import jax
import jax.numpy as jnp
from jax import lax
import jax.experimental.pallas as pl
import jax.experimental.pallas.tpu as pltpu

F32 = jnp.float32
BF16 = jnp.bfloat16
LANES = 128
LOG2E = 1.4426950408889634


def _dot(a, b):
    return lax.dot_general(a, b, (((1,), (0,)), ((), ())), preferred_element_type=F32)


def _dot_nt(a, b):
    return lax.dot_general(a, b, (((1,), (1,)), ((), ())), preferred_element_type=F32)


def _layernorm(x, eps=1e-5):
    m = jnp.mean(x, axis=-1, keepdims=True)
    xc = x - m
    v = jnp.mean(xc * xc, axis=-1, keepdims=True)
    return xc * lax.rsqrt(v + eps)


def _gelu(x):
    c = math.sqrt(2.0 / math.pi)
    return 0.5 * x * (1.0 + jnp.tanh(c * (x + 0.044715 * (x * x * x))))


def _kernel(x_hbm, mem0_ref, wq_hbm, wk_hbm, wv_hbm, wo_hbm, w1_hbm, w2_hbm, w3_hbm, w4_hbm, gw_ref,
            out_hbm,
            x_v, wqkv_v, wo_v, w1_v, w2_v, w3_v, w4_v, stage_v, h_v, b_v, out_v, xsems, wsems,
            *, S, D, H, Dh, M, SEG, TB, NSUB):
    NSEG = S // SEG
    NT = S // TB
    DC = D // NT
    C = D // 4
    HALO = 8

    NJ = D // LANES
    NC = H // 8

    def cp_x(i):
        r0 = pl.multiple_of(i * TB, TB)
        return pltpu.make_async_copy(x_hbm.at[pl.ds(r0, TB), :], x_v.at[pl.ds(r0, TB), :], xsems.at[i])

    def plane(m, parity, c):
        return (m * 2 + parity) * NC + c

    cp_qkv = [
        pltpu.make_async_copy(
            w.bitcast(jnp.uint32).at[:, pl.ds((parity + 2 * half) * (H // 2) + 4 * c, 4), :],
            stage_v.at[plane(m, parity, c), pl.ds(0, D // 4), pl.ds(4 * half, 4), :], wsems.at[4])
        for m, w in enumerate((wq_hbm, wk_hbm, wv_hbm))
        for parity in range(2) for c in range(NC) for half in range(2)]

    def cp_rows(src, dst_u32, sem, pieces):
        dst = dst_u32.bitcast(BF16)
        rows = src.shape[0] // pieces
        return [pltpu.make_async_copy(src.at[pl.ds(t * rows, rows), :], dst.at[pl.ds(t * rows, rows), :], sem)
                for t in range(pieces)]

    cp_w1 = cp_rows(w1_hbm, w1_v, wsems.at[0], 1)
    cp_w2 = cp_rows(w2_hbm, w2_v, wsems.at[1], 1)
    cp_w3 = cp_rows(w3_hbm, w3_v, wsems.at[2], 1)
    cp_w4 = cp_rows(w4_hbm, w4_v, wsems.at[3], 1)
    cp_wo = cp_rows(wo_hbm, wo_v, wsems.at[5], 1)

    cp_x(0).start()
    for c in cp_w1:
        c.start()
    for i in range(1, NT):
        cp_x(i).start()
    for c in cp_w2 + cp_w3 + cp_w4:
        c.start()
    h_v[0:HALO, :] = jnp.zeros((HALO, D), F32)
    h_v[HALO + S:HALO + S + HALO, :] = jnp.zeros((HALO, D), F32)

    TS = TB // NSUB

    def normed_rows(r0):
        return _layernorm(x_v[pl.ds(r0, TS), :].astype(F32)).astype(BF16)

    def b_pass1(i, xn0):
        @pl.when(i + 1 < NT)
        def _():
            cp_x(i + 1).wait()

        rows = [pl.multiple_of(i * TB + t * TS, TS) for t in range(NSUB)]
        xn = [xn0] + [normed_rows(r0) for r0 in rows[1:]]
        for r0, t in zip(rows, xn):
            h_v[pl.ds(r0 + HALO, TS), :] = _gelu(_dot(t, pltpu.bitcast(w1_v[...], BF16)))
        return normed_rows(pl.multiple_of(jnp.minimum(i + 1, NT - 1) * TB, TB))

    cp_x(0).wait()
    xn_first = normed_rows(0)
    for c in cp_w1:
        c.wait()

    lax.fori_loop(0, NT, b_pass1, xn_first)

    for c in cp_qkv + cp_wo:
        c.start()
    for c in cp_w2 + cp_w3:
        c.wait()

    def b_pass2(i, _):
        rows = [pl.multiple_of(i * TB + t * TS, TS) for t in range(NSUB)]
        x1 = []
        for r0 in rows:
            win = h_v[pl.ds(r0, TS + 2 * HALO), :]
            hs_in = jnp.concatenate([
                win[HALO - 1:HALO - 1 + TS, 0 * C:1 * C],
                win[HALO + 1:HALO + 1 + TS, 1 * C:2 * C],
                win[HALO - 2:HALO - 2 + TS, 2 * C:3 * C],
                win[HALO + 2:HALO + 2 + TS, 3 * C:4 * C]], axis=1).astype(BF16)
            x1.append(x_v[pl.ds(r0, TS), :].astype(F32) + _dot(hs_in, pltpu.bitcast(w2_v[...], BF16)))
        u = [_gelu(_dot(_layernorm(t).astype(BF16), pltpu.bitcast(w3_v[...], BF16))).astype(BF16) for t in x1]
        @pl.when(i == 0)
        def _():
            for c in cp_w4:
                c.wait()

        for r0, x1t, ut in zip(rows, x1, u):
            b_v[pl.ds(r0, TS), :] = x1t + _dot(ut, pltpu.bitcast(w4_v[...], BF16))
        return 0

    lax.fori_loop(0, NT, b_pass2, 0)

    for c in cp_qkv + cp_wo:
        c.wait()

    L = M + SEG
    LP = (L + 15) // 16 * 16
    G = 4
    NG = H // G
    row = lax.broadcasted_iota(jnp.int32, (L, LP), 0)
    col = lax.broadcasted_iota(jnp.int32, (L, LP), 1)
    mask = jnp.logical_and(jnp.logical_or(row < M, row >= col), col < L)
    fill = jnp.where(col < L, -1e9 * LOG2E, -jnp.inf).astype(F32)
    qk_scale = (Dh ** -0.5) * LOG2E
    zpad = jnp.zeros((LP - L, Dh), F32)
    gw = gw_ref[...].astype(F32).reshape(1, D)

    def cp_out(s):
        r0 = pl.multiple_of(s * SEG, SEG)
        return pltpu.make_async_copy(out_v.at[pl.ds(r0, SEG), :], out_hbm.at[pl.ds(r0, SEG), :], wsems.at[0])

    stage_2d = stage_v.reshape(6 * NC, (D // 4 + 1) * 8, Dh)

    def project_building(hcat, m, g):
        KW = LANES // 2
        acc = [None] * G
        for kt in range(D // LANES):
            lhs = hcat[:, kt * LANES:(kt + 1) * LANES]
            for t in range(0, G, 2):
                h = g * G + t
                c, r = divmod(h // 2, 4)
                rows = pl.ds(kt * KW * 4 + r, KW, stride=4)
                even = stage_2d[plane(m, 0, c), rows, :]
                odd = stage_2d[plane(m, 1, c), rows, :]
                pair = ((even & jnp.uint32(0xFFFF)) | (odd << 16), (even >> 16) | (odd & jnp.uint32(0xFFFF0000)))
                for n, w in enumerate(pair):
                    wqkv_v[m * H + h + n, kt * KW:(kt + 1) * KW, :] = w
                    part = _dot(lhs, pltpu.bitcast(w, BF16))
                    acc[t + n] = part if kt == 0 else acc[t + n] + part
        return acc

    def project_stored(hcat, m, g):
        return [_dot(hcat, pltpu.bitcast(wqkv_v[m * H + g * G + t], BF16)) for t in range(G)]

    def seg_step(s, mem, project_fn):
        r0 = s * SEG if isinstance(s, int) else pl.multiple_of(s * SEG, SEG)
        xs = x_v[pl.ds(r0, SEG), :].astype(F32)
        hcat = jnp.concatenate([mem, xs], axis=0)

        project = functools.partial(project_fn, hcat)

        def pad_bf16(ts):
            return [jnp.concatenate([t, zpad], axis=0).astype(BF16) for t in ts]

        def softmax(sc):
            t = jnp.where(mask, sc * qk_scale, fill)
            p = jnp.exp2(t - jnp.max(t, axis=-1, keepdims=True))
            l = jnp.sum(p, axis=-1, keepdims=True)
            r = pl.reciprocal(l, approx=True)
            r = r * (2.0 - l * r)
            return p * r

        v, p, o = {}, {}, {}
        acc = [None] * NJ

        def out_proj(g, js):
            ocat = jnp.concatenate(o[g], axis=1)
            k0 = g * G * Dh // 2
            for j in js:
                w = pltpu.bitcast(wo_v[k0:k0 + G * Dh // 2, j * LANES:(j + 1) * LANES], BF16)
                part = _dot(ocat, w)
                acc[j] = part if acc[j] is None else acc[j] + part

        def attend(g):
            o[g] = [_dot(a, b) for a, b in zip(p.pop(g), v.pop(g))]

        for g in range(NG):
            q = project(0, g)
            k = pad_bf16(project(1, g))
            if g >= 1:
                attend(g - 1)
            v[g] = pad_bf16(project(2, g))
            p[g] = [softmax(_dot_nt(a, b)) for a, b in zip(q, k)]
            if g >= 2:
                out_proj(g - 2, range(NJ))
        out_proj(NG - 2, range(NJ // 2))
        attend(NG - 1)
        out_proj(NG - 2, range(NJ // 2, NJ))
        out_proj(NG - 1, range(NJ))
        res = jnp.concatenate(acc, axis=1)
        gate = jax.nn.sigmoid(jnp.sum(xs * gw, axis=-1, keepdims=True))
        out_v[pl.ds(r0, SEG), :] = (gate * res[M:] + (1.0 - gate) * b_v[pl.ds(r0, SEG), :]).astype(BF16)
        return res[:M]

    def later_step(s, mem):
        cp_out(s - 1).start()
        return seg_step(s, mem, project_stored)

    mem1 = seg_step(0, mem0_ref[...].astype(F32), project_building)
    lax.fori_loop(1, NSEG, later_step, mem1)

    cp_out(NSEG - 1).start()
    pltpu.make_async_copy(out_v, out_hbm, wsems.at[0]).wait()


@functools.partial(jax.jit, static_argnames=("A_seg_len",))
def pallas_gated_mix__memory_aug_recurrent_mem_tr__mixer_s_mlp__prompt_kernel(
    A_x: jax.Array,
    A_mem0: jax.Array,
    A_Wq: jax.Array,
    A_Wk: jax.Array,
    A_Wv: jax.Array,
    A_Wo: jax.Array,
    A_seg_len,
    B_x: jax.Array,
    B_w1: jax.Array,
    B_w2: jax.Array,
    B_w3: jax.Array,
    B_w4: jax.Array,
    gate_w: jax.Array,
):
    del B_x
    B, S, D = A_x.shape
    assert B == 1
    _, H, Dh = A_Wq.shape
    M = A_mem0.shape[1]
    SEG = int(A_seg_len)
    Fh = B_w3.shape[1]
    TB = 256

    any_spec = pl.BlockSpec(memory_space=pl.ANY)
    vmem_spec = pl.BlockSpec(memory_space=pltpu.VMEM)
    kernel = functools.partial(_kernel, S=S, D=D, H=H, Dh=Dh, M=M, SEG=SEG, TB=TB, NSUB=2)
    out = pl.pallas_call(
        kernel,
        out_shape=jax.ShapeDtypeStruct((S, D), A_x.dtype),
        in_specs=[any_spec, vmem_spec] + [any_spec] * 8 + [vmem_spec],
        out_specs=any_spec,
        scratch_shapes=[
            pltpu.VMEM((S, D), BF16),
            pltpu.VMEM((3 * H, D // 2, Dh), jnp.uint32),
            pltpu.VMEM((H * Dh // 2, D), jnp.uint32),
            pltpu.VMEM((D // 2, D), jnp.uint32),
            pltpu.VMEM((D // 2, D), jnp.uint32),
            pltpu.VMEM((D // 2, Fh), jnp.uint32),
            pltpu.VMEM((Fh // 2, D), jnp.uint32),
            pltpu.VMEM((6 * H // 8, D // 4 + 1, 8, Dh), jnp.uint32),
            pltpu.VMEM((S + 16, D), F32),
            pltpu.VMEM((S, D), F32),
            pltpu.VMEM((S, D), BF16),
            pltpu.SemaphoreType.DMA((S // TB,)),
            pltpu.SemaphoreType.DMA((6,)),
        ],
        compiler_params=pltpu.CompilerParams(vmem_limit_bytes=124 * 1024 * 1024),
    )(
        A_x.reshape(S, D),
        A_mem0.reshape(M, D),
        A_Wq.reshape(D // 4, 4 * H, Dh),
        A_Wk.reshape(D // 4, 4 * H, Dh),
        A_Wv.reshape(D // 4, 4 * H, Dh),
        A_Wo.reshape(H * Dh, D),
        B_w1, B_w2, B_w3, B_w4,
        gate_w,
    )
    return out.reshape(B, S, D)
```

```python
import functools
import math

import jax
import jax.numpy as jnp
from jax import lax
import jax.experimental.pallas as pl
import jax.experimental.pallas.tpu as pltpu

F32 = jnp.float32
BF16 = jnp.bfloat16
U32 = jnp.uint32
LANES = 128
LOG2E = 1.4426950408889634
HALO = 8
W1_PIECES = 4
HEAD_GROUP = 4


def _dot(a, b):
    return lax.dot_general(a, b, (((1,), (0,)), ((), ())), preferred_element_type=F32)


def _dot_nt(a, b):
    return lax.dot_general(a, b, (((1,), (1,)), ((), ())), preferred_element_type=F32)


def _dot_packed(a, words):
    return _dot(a, pltpu.bitcast(words, BF16))


def _layernorm(x, eps=1e-5):
    xc = x - jnp.mean(x, axis=-1, keepdims=True)
    return xc * lax.rsqrt(jnp.mean(xc * xc, axis=-1, keepdims=True) + eps)


def _gelu(x):
    c = math.sqrt(2.0 / math.pi)
    return 0.5 * x * (1.0 + jnp.tanh(c * (x + 0.044715 * (x * x * x))))


def _kernel(x_hbm, mem0_ref, wq_hbm, wk_hbm, wv_hbm, wo_hbm, w1_hbm, w2_hbm, w3_hbm, w4_hbm, gw_ref,
            out_hbm,
            x_v, wqkv_v, wo_v, w1_v, w2_v, w3_v, w4_v, stage_v, h_v, b_v, out_v, xsems, w1sems, sems,
            *, S, D, H, Dh, M, SEG, TB):
    NSEG = S // SEG
    NT = S // TB
    TS = TB // 2
    C = D // 4
    NJ = D // LANES
    NC = H // 8
    G = HEAD_GROUP
    NG = H // G

    def cp_x(i):
        r0 = pl.multiple_of(i * TB, TB)
        return pltpu.make_async_copy(x_hbm.at[pl.ds(r0, TB), :], x_v.at[pl.ds(r0, TB), :], xsems.at[i])

    w1_cols = [pl.ds(t * (D // W1_PIECES), D // W1_PIECES) for t in range(W1_PIECES)]
    cp_w1 = [pltpu.make_async_copy(w1_hbm.at[:, cols], w1_v.bitcast(BF16).at[:, cols], w1sems.at[t])
             for t, cols in enumerate(w1_cols)]
    cp_w2 = pltpu.make_async_copy(w2_hbm, w2_v.bitcast(BF16), sems.at[0])
    cp_w3 = pltpu.make_async_copy(w3_hbm, w3_v.bitcast(BF16), sems.at[1])
    cp_w4 = pltpu.make_async_copy(w4_hbm, w4_v.bitcast(BF16), sems.at[2])
    cp_wo = pltpu.make_async_copy(wo_hbm, wo_v.bitcast(BF16), sems.at[3])

    def plane(m, parity, c):
        return (m * 2 + parity) * NC + c

    cp_qkv = [
        pltpu.make_async_copy(
            w.bitcast(U32).at[:, pl.ds((parity + 2 * half) * (H // 2) + 4 * c, 4), :],
            stage_v.at[plane(m, parity, c), pl.ds(0, D // 4), pl.ds(4 * half, 4), :], sems.at[4])
        for m, w in enumerate((wq_hbm, wk_hbm, wv_hbm))
        for parity in range(2) for c in range(NC) for half in range(2)]

    def cp_out(s):
        r0 = pl.multiple_of(s * SEG, SEG)
        return pltpu.make_async_copy(out_v.at[pl.ds(r0, SEG), :], out_hbm.at[pl.ds(r0, SEG), :], sems.at[5])

    cp_x(0).start()
    for cp in cp_w1:
        cp.start()
    for i in range(1, NT):
        cp_x(i).start()
    for cp in (cp_w2, cp_w3, cp_w4):
        cp.start()
    h_v[0:HALO, :] = jnp.zeros((HALO, D), F32)
    h_v[HALO + S:HALO + S + HALO, :] = jnp.zeros((HALO, D), F32)

    def tile_rows(i):
        return [pl.multiple_of(i * TB + t * TS, TS) for t in range(2)]

    def normed_rows(r0):
        return _layernorm(x_v[pl.ds(r0, TS), :].astype(F32)).astype(BF16)

    def b_pass1(i, xn_top):
        @pl.when(i + 1 < NT)
        def _():
            cp_x(i + 1).wait()

        rows = tile_rows(i)
        for r0, xn in zip(rows, (xn_top, normed_rows(rows[1]))):
            h_v[pl.ds(r0 + HALO, TS), :] = _gelu(_dot_packed(xn, w1_v[...]))
        return normed_rows(pl.multiple_of(jnp.minimum(i + 1, NT - 1) * TB, TB))

    cp_x(0).wait()
    xn_first = [normed_rows(t * TS) for t in range(2)]
    for cp, cols in zip(cp_w1, w1_cols):
        cp.wait()
        for t, xn in enumerate(xn_first):
            h_v[pl.ds(HALO + t * TS, TS), cols] = _gelu(_dot_packed(xn, w1_v[:, cols]))
    cp_x(1).wait()
    lax.fori_loop(1, NT, b_pass1, normed_rows(TB))

    for cp in cp_qkv + [cp_wo]:
        cp.start()
    cp_w2.wait()
    cp_w3.wait()

    def b_pass2(i, _):
        rows = tile_rows(i)
        x1 = []
        for r0 in rows:
            win = h_v[pl.ds(r0, TS + 2 * HALO), :]
            shifted = jnp.concatenate([
                win[HALO - 1:HALO - 1 + TS, 0 * C:1 * C],
                win[HALO + 1:HALO + 1 + TS, 1 * C:2 * C],
                win[HALO - 2:HALO - 2 + TS, 2 * C:3 * C],
                win[HALO + 2:HALO + 2 + TS, 3 * C:4 * C]], axis=1).astype(BF16)
            x1.append(x_v[pl.ds(r0, TS), :].astype(F32) + _dot_packed(shifted, w2_v[...]))
        u = [_gelu(_dot_packed(_layernorm(t).astype(BF16), w3_v[...])).astype(BF16) for t in x1]

        @pl.when(i == 0)
        def _():
            cp_w4.wait()

        for r0, x1t, ut in zip(rows, x1, u):
            b_v[pl.ds(r0, TS), :] = x1t + _dot_packed(ut, w4_v[...])
        return 0

    lax.fori_loop(0, NT, b_pass2, 0)

    for cp in cp_qkv + [cp_wo]:
        cp.wait()

    L = M + SEG
    LP = (L + 15) // 16 * 16
    qk_scale = (Dh ** -0.5) * LOG2E
    zpad = jnp.zeros((LP - L, Dh), F32)
    gw = gw_ref[...].astype(F32).reshape(1, D)
    stage_2d = stage_v.reshape(6 * NC, (D // 4 + 1) * 8, Dh)

    row = lax.broadcasted_iota(jnp.int32, (L, LP), 0)
    col = lax.broadcasted_iota(jnp.int32, (L, LP), 1)
    keep = jnp.logical_and(jnp.logical_or(row < M, row >= col), col < L)
    fill = jnp.where(col < L, -1e9 * LOG2E, -jnp.inf).astype(F32)

    def project_building(lhs, m, g):
        KW = LANES // 2
        acc = [None] * G
        for kt in range(D // LANES):
            lhs_k = lhs[:, kt * LANES:(kt + 1) * LANES]
            for t in range(0, G, 2):
                h = g * G + t
                c, r = divmod(h // 2, 4)
                rows = pl.ds(kt * KW * 4 + r, KW, stride=4)
                even = stage_2d[plane(m, 0, c), rows, :]
                odd = stage_2d[plane(m, 1, c), rows, :]
                pair = ((even & U32(0xFFFF)) | (odd << 16), (even >> 16) | (odd & U32(0xFFFF0000)))
                for n, words in enumerate(pair):
                    wqkv_v[m * H + h + n, kt * KW:(kt + 1) * KW, :] = words
                    part = _dot_packed(lhs_k, words)
                    acc[t + n] = part if kt == 0 else acc[t + n] + part
        return acc

    def project_stored(lhs, m, g):
        return [_dot_packed(lhs, wqkv_v[m * H + g * G + t]) for t in range(G)]

    def seg_step(s, mem, project):
        r0 = s * SEG if isinstance(s, int) else pl.multiple_of(s * SEG, SEG)
        xs = x_v[pl.ds(r0, SEG), :].astype(F32)
        hcat = jnp.concatenate([mem, xs], axis=0)

        def pad_bf16(ts):
            return [jnp.concatenate([t, zpad], axis=0).astype(BF16) for t in ts]

        def softmax(scores):
            t = jnp.where(keep, scores * qk_scale, fill)
            e = jnp.exp2(t - jnp.max(t, axis=-1, keepdims=True))
            total = jnp.sum(e, axis=-1, keepdims=True)
            inv = pl.reciprocal(total, approx=True)
            inv = inv * (2.0 - total * inv)
            return e * inv

        v, p, o = {}, {}, {}
        acc = [None] * NJ

        def attend(g):
            o[g] = [_dot(a, b) for a, b in zip(p.pop(g), v.pop(g))]

        def out_proj(g, js):
            ocat = jnp.concatenate(o[g], axis=1)
            k0 = g * G * Dh // 2
            for j in js:
                part = _dot_packed(ocat, wo_v[k0:k0 + G * Dh // 2, j * LANES:(j + 1) * LANES])
                acc[j] = part if acc[j] is None else acc[j] + part

        for g in range(NG):
            q = project(hcat, 0, g)
            k = pad_bf16(project(hcat, 1, g))
            if g >= 1:
                attend(g - 1)
            v[g] = pad_bf16(project(hcat, 2, g))
            p[g] = [softmax(_dot_nt(a, b)) for a, b in zip(q, k)]
            if g >= 2:
                out_proj(g - 2, range(NJ))
        out_proj(NG - 2, range(NJ // 2))
        attend(NG - 1)
        out_proj(NG - 2, range(NJ // 2, NJ))
        out_proj(NG - 1, range(NJ))
        res = jnp.concatenate(acc, axis=1)
        gate = jax.nn.sigmoid(jnp.sum(xs * gw, axis=-1, keepdims=True))
        out_v[pl.ds(r0, SEG), :] = (gate * res[M:] + (1.0 - gate) * b_v[pl.ds(r0, SEG), :]).astype(BF16)
        return res[:M]

    def later_step(s, mem):
        cp_out(s - 1).start()
        return seg_step(s, mem, project_stored)

    mem = seg_step(0, mem0_ref[...].astype(F32), project_building)
    lax.fori_loop(1, NSEG, later_step, mem)
    cp_out(NSEG - 1).start()
    pltpu.make_async_copy(out_v, out_hbm, sems.at[5]).wait()


@functools.partial(jax.jit, static_argnames=("A_seg_len",))
def pallas_gated_mix__memory_aug_recurrent_mem_tr__mixer_s_mlp__prompt_kernel(
    A_x: jax.Array,
    A_mem0: jax.Array,
    A_Wq: jax.Array,
    A_Wk: jax.Array,
    A_Wv: jax.Array,
    A_Wo: jax.Array,
    A_seg_len,
    B_x: jax.Array,
    B_w1: jax.Array,
    B_w2: jax.Array,
    B_w3: jax.Array,
    B_w4: jax.Array,
    gate_w: jax.Array,
):
    del B_x
    B, S, D = A_x.shape
    _, H, Dh = A_Wq.shape
    M = A_mem0.shape[1]
    SEG = int(A_seg_len)
    Fh = B_w3.shape[1]
    TB = 256
    assert B == 1 and Dh == LANES and S % TB == 0 and S % SEG == 0 and H % 8 == 0 and D % (4 * LANES) == 0

    any_spec = pl.BlockSpec(memory_space=pl.ANY)
    vmem_spec = pl.BlockSpec(memory_space=pltpu.VMEM)
    kernel = functools.partial(_kernel, S=S, D=D, H=H, Dh=Dh, M=M, SEG=SEG, TB=TB)
    out = pl.pallas_call(
        kernel,
        out_shape=jax.ShapeDtypeStruct((S, D), A_x.dtype),
        in_specs=[any_spec, vmem_spec] + [any_spec] * 8 + [vmem_spec],
        out_specs=any_spec,
        scratch_shapes=[
            pltpu.VMEM((S, D), BF16),
            pltpu.VMEM((3 * H, D // 2, Dh), U32),
            pltpu.VMEM((H * Dh // 2, D), U32),
            pltpu.VMEM((D // 2, D), U32),
            pltpu.VMEM((D // 2, D), U32),
            pltpu.VMEM((D // 2, Fh), U32),
            pltpu.VMEM((Fh // 2, D), U32),
            pltpu.VMEM((6 * H // 8, D // 4 + 1, 8, Dh), U32),
            pltpu.VMEM((S + 2 * HALO, D), F32),
            pltpu.VMEM((S, D), F32),
            pltpu.VMEM((S, D), BF16),
            pltpu.SemaphoreType.DMA((S // TB,)),
            pltpu.SemaphoreType.DMA((W1_PIECES,)),
            pltpu.SemaphoreType.DMA((6,)),
        ],
        compiler_params=pltpu.CompilerParams(vmem_limit_bytes=124 * 1024 * 1024),
    )(
        A_x.reshape(S, D),
        A_mem0.reshape(M, D),
        A_Wq.reshape(D // 4, 4 * H, Dh),
        A_Wk.reshape(D // 4, 4 * H, Dh),
        A_Wv.reshape(D // 4, 4 * H, Dh),
        A_Wo.reshape(H * Dh, D),
        B_w1, B_w2, B_w3, B_w4,
        gate_w,
    )
    return out.reshape(B, S, D)
```

```python
import functools
import math

import jax
import jax.numpy as jnp
from jax import lax
import jax.experimental.pallas as pl
import jax.experimental.pallas.tpu as pltpu

F32 = jnp.float32
BF16 = jnp.bfloat16
U32 = jnp.uint32
LANES = 128
LOG2E = 1.4426950408889634
HALO = 8
W1_PIECES = 4
HEAD_GROUP = 4


def _dot(a, b):
    return lax.dot_general(a, b, (((1,), (0,)), ((), ())), preferred_element_type=F32)


def _dot_nt(a, b):
    return lax.dot_general(a, b, (((1,), (1,)), ((), ())), preferred_element_type=F32)


def _dot_packed(a, words):
    return _dot(a, pltpu.bitcast(words, BF16))


def _layernorm(x, eps=1e-5):
    xc = x - jnp.mean(x, axis=-1, keepdims=True)
    return xc * lax.rsqrt(jnp.mean(xc * xc, axis=-1, keepdims=True) + eps)


def _gelu(x):
    c = math.sqrt(2.0 / math.pi)
    return 0.5 * x * (1.0 + jnp.tanh(c * (x + 0.044715 * (x * x * x))))


def _kernel(x_hbm, mem0_hbm, wq_hbm, wk_hbm, wv_hbm, wo_hbm, w1_hbm, w2_hbm, w3_hbm, w4_hbm, gw_hbm,
            out_hbm,
            x_v, wqkv_v, wo_v, w1_v, w2_v, w3_v, w4_v, stage_v, h_v, b_v, out_v, mem0_v, gw_v, xsems, w1sems, sems,
            *, S, D, H, Dh, M, SEG, TB):
    NSEG = S // SEG
    NT = S // TB
    TS = TB // 2
    C = D // 4
    NJ = D // LANES
    NC = H // 8
    G = HEAD_GROUP
    NG = H // G

    def cp_x(i):
        r0 = pl.multiple_of(i * TB, TB)
        return pltpu.make_async_copy(x_hbm.at[pl.ds(r0, TB), :], x_v.at[pl.ds(r0, TB), :], xsems.at[i])

    w1_cols = [pl.ds(t * (D // W1_PIECES), D // W1_PIECES) for t in range(W1_PIECES)]
    cp_w1 = [pltpu.make_async_copy(w1_hbm.at[:, cols], w1_v.bitcast(BF16).at[:, cols], w1sems.at[t])
             for t, cols in enumerate(w1_cols)]
    cp_w2 = pltpu.make_async_copy(w2_hbm, w2_v.bitcast(BF16), sems.at[0])
    cp_w3 = pltpu.make_async_copy(w3_hbm, w3_v.bitcast(BF16), sems.at[1])
    cp_w4 = pltpu.make_async_copy(w4_hbm, w4_v.bitcast(BF16), sems.at[2])
    cp_wo = pltpu.make_async_copy(wo_hbm, wo_v.bitcast(BF16), sems.at[3])

    def plane(m, parity, c):
        return (m * 2 + parity) * NC + c

    cp_qkv = [
        pltpu.make_async_copy(
            w.bitcast(U32).at[:, pl.ds((parity + 2 * half) * (H // 2) + 4 * c, 4), :],
            stage_v.at[plane(m, parity, c), pl.ds(0, D // 4), pl.ds(4 * half, 4), :], sems.at[4])
        for m, w in enumerate((wq_hbm, wk_hbm, wv_hbm))
        for parity in range(2) for c in range(NC) for half in range(2)]

    cp_a = cp_qkv + [cp_wo, pltpu.make_async_copy(mem0_hbm, mem0_v, sems.at[6]),
                     pltpu.make_async_copy(gw_hbm, gw_v, sems.at[7])]

    def cp_out(s):
        r0 = pl.multiple_of(s * SEG, SEG)
        return pltpu.make_async_copy(out_v.at[pl.ds(r0, SEG), :], out_hbm.at[pl.ds(r0, SEG), :], sems.at[5])

    cp_x(0).start()
    for cp in cp_w1:
        cp.start()
    for i in range(1, NT):
        cp_x(i).start()
    for cp in (cp_w2, cp_w3, cp_w4):
        cp.start()
    h_v[0:HALO, :] = jnp.zeros((HALO, D), F32)
    h_v[HALO + S:HALO + S + HALO, :] = jnp.zeros((HALO, D), F32)

    def tile_rows(i):
        return [pl.multiple_of(i * TB + t * TS, TS) for t in range(2)]

    def normed_rows(r0):
        return _layernorm(x_v[pl.ds(r0, TS), :].astype(F32)).astype(BF16)

    def b_pass1(i, xn_top):
        @pl.when(i + 1 < NT)
        def _():
            cp_x(i + 1).wait()

        rows = tile_rows(i)
        for r0, xn in zip(rows, (xn_top, normed_rows(rows[1]))):
            h_v[pl.ds(r0 + HALO, TS), :] = _gelu(_dot_packed(xn, w1_v[...]))
        return normed_rows(pl.multiple_of(jnp.minimum(i + 1, NT - 1) * TB, TB))

    cp_x(0).wait()
    xn_first = [normed_rows(t * TS) for t in range(2)]
    for cp, cols in zip(cp_w1, w1_cols):
        cp.wait()
        for t, xn in enumerate(xn_first):
            h_v[pl.ds(HALO + t * TS, TS), cols] = _gelu(_dot_packed(xn, w1_v[:, cols]))
    cp_x(1).wait()
    lax.fori_loop(1, NT, b_pass1, normed_rows(TB))

    for cp in cp_a:
        cp.start()
    cp_w2.wait()
    cp_w3.wait()

    def b_pass2(i, _):
        rows = tile_rows(i)
        x1 = []
        for r0 in rows:
            win = h_v[pl.ds(r0, TS + 2 * HALO), :]
            shifted = jnp.concatenate([
                win[HALO - 1:HALO - 1 + TS, 0 * C:1 * C],
                win[HALO + 1:HALO + 1 + TS, 1 * C:2 * C],
                win[HALO - 2:HALO - 2 + TS, 2 * C:3 * C],
                win[HALO + 2:HALO + 2 + TS, 3 * C:4 * C]], axis=1).astype(BF16)
            x1.append(x_v[pl.ds(r0, TS), :].astype(F32) + _dot_packed(shifted, w2_v[...]))
        u = [_gelu(_dot_packed(_layernorm(t).astype(BF16), w3_v[...])).astype(BF16) for t in x1]

        @pl.when(i == 0)
        def _():
            cp_w4.wait()

        for r0, x1t, ut in zip(rows, x1, u):
            b_v[pl.ds(r0, TS), :] = x1t + _dot_packed(ut, w4_v[...])
        return 0

    lax.fori_loop(0, NT, b_pass2, 0)

    for cp in cp_a:
        cp.wait()

    L = M + SEG
    LP = (L + 15) // 16 * 16
    qk_scale = (Dh ** -0.5) * LOG2E
    zpad = jnp.zeros((LP - L, Dh), F32)
    gw = gw_v[...].astype(F32).reshape(1, D)
    stage_2d = stage_v.reshape(6 * NC, (D // 4 + 1) * 8, Dh)

    row = lax.broadcasted_iota(jnp.int32, (L, LP), 0)
    col = lax.broadcasted_iota(jnp.int32, (L, LP), 1)
    keep = jnp.logical_and(jnp.logical_or(row < M, row >= col), col < L)
    fill = jnp.where(col < L, -1e9 * LOG2E, -jnp.inf).astype(F32)

    def project_building(lhs, m, g):
        KW = LANES // 2
        acc = [None] * G
        for kt in range(D // LANES):
            lhs_k = lhs[:, kt * LANES:(kt + 1) * LANES]
            for t in range(0, G, 2):
                h = g * G + t
                c, r = divmod(h // 2, 4)
                rows = pl.ds(kt * KW * 4 + r, KW, stride=4)
                even = stage_2d[plane(m, 0, c), rows, :]
                odd = stage_2d[plane(m, 1, c), rows, :]
                pair = ((even & U32(0xFFFF)) | (odd << 16), (even >> 16) | (odd & U32(0xFFFF0000)))
                for n, words in enumerate(pair):
                    wqkv_v[m * H + h + n, kt * KW:(kt + 1) * KW, :] = words
                    part = _dot_packed(lhs_k, words)
                    acc[t + n] = part if kt == 0 else acc[t + n] + part
        return acc

    def project_stored(lhs, m, g):
        return [_dot_packed(lhs, wqkv_v[m * H + g * G + t]) for t in range(G)]

    def seg_step(s, mem, project):
        r0 = s * SEG if isinstance(s, int) else pl.multiple_of(s * SEG, SEG)
        xs = x_v[pl.ds(r0, SEG), :].astype(F32)
        hcat = jnp.concatenate([mem, xs], axis=0)

        def pad_bf16(ts):
            return [jnp.concatenate([t, zpad], axis=0).astype(BF16) for t in ts]

        def softmax(scores):
            t = jnp.where(keep, scores * qk_scale, fill)
            e = jnp.exp2(t - jnp.max(t, axis=-1, keepdims=True))
            total = jnp.sum(e, axis=-1, keepdims=True)
            inv = pl.reciprocal(total, approx=True)
            inv = inv * (2.0 - total * inv)
            return e * inv

        v, p, o = {}, {}, {}
        acc = [None] * NJ

        def attend(g):
            o[g] = [_dot(a, b) for a, b in zip(p.pop(g), v.pop(g))]

        def out_proj(g, js):
            ocat = jnp.concatenate(o[g], axis=1)
            k0 = g * G * Dh // 2
            for j in js:
                part = _dot_packed(ocat, wo_v[k0:k0 + G * Dh // 2, j * LANES:(j + 1) * LANES])
                acc[j] = part if acc[j] is None else acc[j] + part

        for g in range(NG):
            q = project(hcat, 0, g)
            k = pad_bf16(project(hcat, 1, g))
            if g >= 1:
                attend(g - 1)
            v[g] = pad_bf16(project(hcat, 2, g))
            p[g] = [softmax(_dot_nt(a, b)) for a, b in zip(q, k)]
            if g >= 2:
                out_proj(g - 2, range(NJ))
        out_proj(NG - 2, range(NJ // 2))
        attend(NG - 1)
        out_proj(NG - 2, range(NJ // 2, NJ))
        out_proj(NG - 1, range(NJ))
        res = jnp.concatenate(acc, axis=1)
        gate = jax.nn.sigmoid(jnp.sum(xs * gw, axis=-1, keepdims=True))
        out_v[pl.ds(r0, SEG), :] = (gate * res[M:] + (1.0 - gate) * b_v[pl.ds(r0, SEG), :]).astype(BF16)
        return res[:M]

    def later_step(s, mem):
        cp_out(s - 1).start()
        return seg_step(s, mem, project_stored)

    mem = seg_step(0, mem0_v[...].astype(F32), project_building)
    lax.fori_loop(1, NSEG, later_step, mem)
    cp_out(NSEG - 1).start()
    pltpu.make_async_copy(out_v, out_hbm, sems.at[5]).wait()


@functools.partial(jax.jit, static_argnames=("A_seg_len",))
def pallas_gated_mix__memory_aug_recurrent_mem_tr__mixer_s_mlp__prompt_kernel(
    A_x: jax.Array,
    A_mem0: jax.Array,
    A_Wq: jax.Array,
    A_Wk: jax.Array,
    A_Wv: jax.Array,
    A_Wo: jax.Array,
    A_seg_len,
    B_x: jax.Array,
    B_w1: jax.Array,
    B_w2: jax.Array,
    B_w3: jax.Array,
    B_w4: jax.Array,
    gate_w: jax.Array,
):
    del B_x
    B, S, D = A_x.shape
    _, H, Dh = A_Wq.shape
    M = A_mem0.shape[1]
    SEG = int(A_seg_len)
    Fh = B_w3.shape[1]
    TB = 256
    assert B == 1 and Dh == LANES and S % TB == 0 and S % SEG == 0 and H % 8 == 0 and D % (4 * LANES) == 0

    any_spec = pl.BlockSpec(memory_space=pl.ANY)
    kernel = functools.partial(_kernel, S=S, D=D, H=H, Dh=Dh, M=M, SEG=SEG, TB=TB)
    out = pl.pallas_call(
        kernel,
        out_shape=jax.ShapeDtypeStruct((S, D), A_x.dtype),
        in_specs=[any_spec] * 11,
        out_specs=any_spec,
        scratch_shapes=[
            pltpu.VMEM((S, D), BF16),
            pltpu.VMEM((3 * H, D // 2, Dh), U32),
            pltpu.VMEM((H * Dh // 2, D), U32),
            pltpu.VMEM((D // 2, D), U32),
            pltpu.VMEM((D // 2, D), U32),
            pltpu.VMEM((D // 2, Fh), U32),
            pltpu.VMEM((Fh // 2, D), U32),
            pltpu.VMEM((6 * H // 8, D // 4 + 1, 8, Dh), U32),
            pltpu.VMEM((S + 2 * HALO, D), F32),
            pltpu.VMEM((S, D), F32),
            pltpu.VMEM((S, D), BF16),
            pltpu.VMEM((M, D), BF16),
            pltpu.VMEM((D,), BF16),
            pltpu.SemaphoreType.DMA((S // TB,)),
            pltpu.SemaphoreType.DMA((W1_PIECES,)),
            pltpu.SemaphoreType.DMA((8,)),
        ],
        compiler_params=pltpu.CompilerParams(vmem_limit_bytes=124 * 1024 * 1024),
    )(
        A_x.reshape(S, D),
        A_mem0.reshape(M, D),
        A_Wq.reshape(D // 4, 4 * H, Dh),
        A_Wk.reshape(D // 4, 4 * H, Dh),
        A_Wv.reshape(D // 4, 4 * H, Dh),
        A_Wo.reshape(H * Dh, D),
        B_w1, B_w2, B_w3, B_w4,
        gate_w,
    )
    return out.reshape(B, S, D)
```

```python
import functools
import math

import jax
import jax.numpy as jnp
import numpy as np
from jax import lax
import jax.experimental.pallas as pl
import jax.experimental.pallas.tpu as pltpu

F32 = jnp.float32
BF16 = jnp.bfloat16
U32 = jnp.uint32
LANES = 128
LOG2E = 1.4426950408889634
LOW_HALF = np.uint32(0x0000FFFF)
HIGH_HALF = np.uint32(0xFFFF0000)
HALO = 8
W1_PIECES = 4
HEAD_GROUP = 4


def _dot(a, b):
    return lax.dot_general(a, b, (((1,), (0,)), ((), ())), preferred_element_type=F32)


def _dot_nt(a, b):
    return lax.dot_general(a, b, (((1,), (1,)), ((), ())), preferred_element_type=F32)


def _dot_packed(a, words):
    return _dot(a, pltpu.bitcast(words, BF16))


def _layernorm(x, eps=1e-5):
    xc = x - jnp.mean(x, axis=-1, keepdims=True)
    return xc * lax.rsqrt(jnp.mean(xc * xc, axis=-1, keepdims=True) + eps)


def _gelu(x):
    c = math.sqrt(2.0 / math.pi)
    return 0.5 * x * (1.0 + jnp.tanh(c * (x + 0.044715 * (x * x * x))))


def _kernel(x_hbm, mem0_hbm, wq_hbm, wk_hbm, wv_hbm, wo_hbm, w1_hbm, w2_hbm, w3_hbm, w4_hbm, gw_hbm,
            out_hbm,
            x_v, wqkv_v, wo_v, w1_v, w2_v, w3_v, w4_v, stage_v, h_v, b_v, out_v, mem0_v, gw_v, xsems, w1sems, sems,
            *, S, D, H, Dh, M, SEG, TB):
    NSEG = S // SEG
    NT = S // TB
    TS = TB // 2
    C = D // 4
    NJ = D // LANES
    NC = H // 8
    G = HEAD_GROUP
    NG = H // G

    def cp_x(i):
        r0 = pl.multiple_of(i * TB, TB)
        return pltpu.make_async_copy(x_hbm.at[pl.ds(r0, TB), :], x_v.at[pl.ds(r0, TB), :], xsems.at[i])

    w1_cols = [pl.ds(t * (D // W1_PIECES), D // W1_PIECES) for t in range(W1_PIECES)]
    cp_w1 = [pltpu.make_async_copy(w1_hbm.at[:, cols], w1_v.bitcast(BF16).at[t], w1sems.at[t])
             for t, cols in enumerate(w1_cols)]
    cp_w2 = pltpu.make_async_copy(w2_hbm, w2_v.bitcast(BF16), sems.at[0])
    cp_w3 = pltpu.make_async_copy(w3_hbm, w3_v.bitcast(BF16), sems.at[1])
    cp_w4 = pltpu.make_async_copy(w4_hbm, w4_v.bitcast(BF16), sems.at[2])
    cp_wo = pltpu.make_async_copy(wo_hbm, wo_v.bitcast(BF16), sems.at[3])

    def plane(m, parity, c):
        return (m * 2 + parity) * NC + c

    cp_qkv = [
        pltpu.make_async_copy(
            w.bitcast(U32).at[:, pl.ds((parity + 2 * half) * (H // 2) + 4 * c, 4), :],
            stage_v.at[plane(m, parity, c), pl.ds(0, D // 4), pl.ds(4 * half, 4), :], sems.at[4])
        for m, w in enumerate((wq_hbm, wk_hbm, wv_hbm))
        for parity in range(2) for c in range(NC) for half in range(2)]

    cp_a = cp_qkv + [cp_wo, pltpu.make_async_copy(mem0_hbm, mem0_v, sems.at[6]),
                     pltpu.make_async_copy(gw_hbm, gw_v, sems.at[7])]

    def cp_out(s):
        r0 = pl.multiple_of(s * SEG, SEG)
        return pltpu.make_async_copy(out_v.at[pl.ds(r0, SEG), :], out_hbm.at[pl.ds(r0, SEG), :], sems.at[5])

    cp_x(0).start()
    for cp in cp_w1:
        cp.start()
    for i in range(1, NT):
        cp_x(i).start()
    for cp in (cp_w2, cp_w3, cp_w4):
        cp.start()
    h_v[0:HALO, :] = jnp.zeros((HALO, D), F32)
    h_v[HALO + S:HALO + S + HALO, :] = jnp.zeros((HALO, D), F32)

    def tile_rows(i):
        return [pl.multiple_of(i * TB + t * TS, TS) for t in range(2)]

    def normed_rows(r0):
        return _layernorm(x_v[pl.ds(r0, TS), :].astype(F32)).astype(BF16)

    def b_pass1(i, xn_top):
        @pl.when(i + 1 < NT)
        def _():
            cp_x(i + 1).wait()

        rows = tile_rows(i)
        w1 = jnp.concatenate([w1_v[t] for t in range(W1_PIECES)], axis=1)
        for r0, xn in zip(rows, (xn_top, normed_rows(rows[1]))):
            h_v[pl.ds(r0 + HALO, TS), :] = _gelu(_dot_packed(xn, w1))
        return normed_rows(pl.multiple_of(jnp.minimum(i + 1, NT - 1) * TB, TB))

    cp_x(0).wait()
    xn_first = [normed_rows(t * TS) for t in range(2)]
    for piece, (cp, cols) in enumerate(zip(cp_w1, w1_cols)):
        cp.wait()
        for t, xn in enumerate(xn_first):
            h_v[pl.ds(HALO + t * TS, TS), cols] = _gelu(_dot_packed(xn, w1_v[piece]))
    cp_x(1).wait()
    lax.fori_loop(1, NT, b_pass1, normed_rows(TB))

    for cp in cp_a:
        cp.start()
    cp_w2.wait()
    cp_w3.wait()

    def b_pass2(i, _):
        rows = tile_rows(i)
        x1 = []
        for r0 in rows:
            win = h_v[pl.ds(r0, TS + 2 * HALO), :]
            shifted = jnp.concatenate([
                win[HALO - 1:HALO - 1 + TS, 0 * C:1 * C],
                win[HALO + 1:HALO + 1 + TS, 1 * C:2 * C],
                win[HALO - 2:HALO - 2 + TS, 2 * C:3 * C],
                win[HALO + 2:HALO + 2 + TS, 3 * C:4 * C]], axis=1).astype(BF16)
            x1.append(x_v[pl.ds(r0, TS), :].astype(F32) + _dot_packed(shifted, w2_v[...]))
        u = [_gelu(_dot_packed(_layernorm(t).astype(BF16), w3_v[...])).astype(BF16) for t in x1]

        @pl.when(i == 0)
        def _():
            cp_w4.wait()

        for r0, x1t, ut in zip(rows, x1, u):
            b_v[pl.ds(r0, TS), :] = x1t + _dot_packed(ut, w4_v[...])
        return 0

    lax.fori_loop(0, NT, b_pass2, 0)

    for cp in cp_a:
        cp.wait()

    L = M + SEG
    LP = (L + 15) // 16 * 16
    qk_scale = (Dh ** -0.5) * LOG2E
    zpad = jnp.zeros((LP - L, Dh), F32)
    gw = gw_v[...].astype(F32).reshape(1, D)
    stage_2d = stage_v.reshape(6 * NC, (D // 4 + 1) * 8, Dh)

    row = lax.broadcasted_iota(jnp.int32, (L, LP), 0)
    col = lax.broadcasted_iota(jnp.int32, (L, LP), 1)
    keep = jnp.logical_and(jnp.logical_or(row < M, row >= col), col < L)
    fill = jnp.where(col < L, -1e9 * LOG2E, -jnp.inf).astype(F32)

    def project_building(lhs, m, g):
        KW = LANES // 2
        acc = [None] * G
        for kt in range(D // LANES):
            lhs_k = lhs[:, kt * LANES:(kt + 1) * LANES]
            for t in range(0, G, 2):
                h = g * G + t
                c, r = divmod(h // 2, 4)
                rows = pl.ds(kt * KW * 4 + r, KW, stride=4)
                even = stage_2d[plane(m, 0, c), rows, :]
                odd = stage_2d[plane(m, 1, c), rows, :]
                pair = ((even & LOW_HALF) | (odd << 16), (even >> 16) | (odd & HIGH_HALF))
                for n, words in enumerate(pair):
                    wqkv_v[m * H + h + n, kt * KW:(kt + 1) * KW, :] = words
                    part = _dot_packed(lhs_k, words)
                    acc[t + n] = part if kt == 0 else acc[t + n] + part
        return acc

    def project_stored(lhs, m, g):
        return [_dot_packed(lhs, wqkv_v[m * H + g * G + t]) for t in range(G)]

    def seg_step(s, mem, project):
        r0 = s * SEG if isinstance(s, int) else pl.multiple_of(s * SEG, SEG)
        xs = x_v[pl.ds(r0, SEG), :].astype(F32)
        hcat = jnp.concatenate([mem, xs], axis=0)

        def pad_bf16(ts):
            return [jnp.concatenate([t, zpad], axis=0).astype(BF16) for t in ts]

        def softmax(scores):
            t = jnp.where(keep, scores * qk_scale, fill)
            e = jnp.exp2(t - jnp.max(t, axis=-1, keepdims=True))
            total = jnp.sum(e, axis=-1, keepdims=True)
            inv = pl.reciprocal(total, approx=True)
            inv = inv * (2.0 - total * inv)
            return e * inv

        v, p, o = {}, {}, {}
        acc = [None] * NJ

        def attend(g):
            o[g] = [_dot(a, b) for a, b in zip(p.pop(g), v.pop(g))]

        def out_proj(g, js):
            ocat = jnp.concatenate(o[g], axis=1)
            k0 = g * G * Dh // 2
            for j in js:
                part = _dot_packed(ocat, wo_v[k0:k0 + G * Dh // 2, j * LANES:(j + 1) * LANES])
                acc[j] = part if acc[j] is None else acc[j] + part

        for g in range(NG):
            q = project(hcat, 0, g)
            k = pad_bf16(project(hcat, 1, g))
            if g >= 1:
                attend(g - 1)
            v[g] = pad_bf16(project(hcat, 2, g))
            p[g] = [softmax(_dot_nt(a, b)) for a, b in zip(q, k)]
            if g >= 2:
                out_proj(g - 2, range(NJ))
        out_proj(NG - 2, range(NJ // 2))
        attend(NG - 1)
        out_proj(NG - 2, range(NJ // 2, NJ))
        out_proj(NG - 1, range(NJ))
        res = jnp.concatenate(acc, axis=1)
        gate = jax.nn.sigmoid(jnp.sum(xs * gw, axis=-1, keepdims=True))
        out_v[pl.ds(r0, SEG), :] = (gate * res[M:] + (1.0 - gate) * b_v[pl.ds(r0, SEG), :]).astype(BF16)
        return res[:M]

    def later_step(s, mem):
        cp_out(s - 1).start()
        return seg_step(s, mem, project_stored)

    mem = seg_step(0, mem0_v[...].astype(F32), project_building)
    lax.fori_loop(1, NSEG, later_step, mem)
    cp_out(NSEG - 1).start()
    pltpu.make_async_copy(out_v, out_hbm, sems.at[5]).wait()


@functools.partial(jax.jit, static_argnames=("A_seg_len",))
def pallas_gated_mix__memory_aug_recurrent_mem_tr__mixer_s_mlp__prompt_kernel(
    A_x: jax.Array,
    A_mem0: jax.Array,
    A_Wq: jax.Array,
    A_Wk: jax.Array,
    A_Wv: jax.Array,
    A_Wo: jax.Array,
    A_seg_len,
    B_x: jax.Array,
    B_w1: jax.Array,
    B_w2: jax.Array,
    B_w3: jax.Array,
    B_w4: jax.Array,
    gate_w: jax.Array,
):
    del B_x
    B, S, D = A_x.shape
    _, H, Dh = A_Wq.shape
    M = A_mem0.shape[1]
    SEG = int(A_seg_len)
    Fh = B_w3.shape[1]
    TB = 256
    assert B == 1 and Dh == LANES and S % TB == 0 and S % SEG == 0 and H % 8 == 0 and D % (4 * LANES) == 0

    any_spec = pl.BlockSpec(memory_space=pl.ANY)
    kernel = functools.partial(_kernel, S=S, D=D, H=H, Dh=Dh, M=M, SEG=SEG, TB=TB)
    out = pl.pallas_call(
        kernel,
        out_shape=jax.ShapeDtypeStruct((S, D), A_x.dtype),
        in_specs=[any_spec] * 11,
        out_specs=any_spec,
        scratch_shapes=[
            pltpu.VMEM((S, D), BF16),
            pltpu.VMEM((3 * H, D // 2, Dh), U32),
            pltpu.VMEM((H * Dh // 2, D), U32),
            pltpu.VMEM((W1_PIECES, D // 2, D // W1_PIECES), U32),
            pltpu.VMEM((D // 2, D), U32),
            pltpu.VMEM((D // 2, Fh), U32),
            pltpu.VMEM((Fh // 2, D), U32),
            pltpu.VMEM((6 * H // 8, D // 4 + 1, 8, Dh), U32),
            pltpu.VMEM((S + 2 * HALO, D), F32),
            pltpu.VMEM((S, D), F32),
            pltpu.VMEM((S, D), BF16),
            pltpu.VMEM((M, D), BF16),
            pltpu.VMEM((D,), BF16),
            pltpu.SemaphoreType.DMA((S // TB,)),
            pltpu.SemaphoreType.DMA((W1_PIECES,)),
            pltpu.SemaphoreType.DMA((8,)),
        ],
        compiler_params=pltpu.CompilerParams(vmem_limit_bytes=124 * 1024 * 1024),
    )(
        A_x.reshape(S, D),
        A_mem0.reshape(M, D),
        A_Wq.reshape(D // 4, 4 * H, Dh),
        A_Wk.reshape(D // 4, 4 * H, Dh),
        A_Wv.reshape(D // 4, 4 * H, Dh),
        A_Wo.reshape(H * Dh, D),
        B_w1, B_w2, B_w3, B_w4,
        gate_w,
    )
    return out.reshape(B, S, D)
```
